```python
import os as _os
_os.environ.setdefault("JAX_PLATFORMS", "cpu")
import jax
import jax.numpy as jnp

def _softmax(x, axis=-1):
    return jax.nn.softmax(x, axis=axis)
def _gelu(x):
    return jax.nn.gelu(x, approximate=True)
def _silu(x):
    return jax.nn.silu(x)
def _sigmoid(x):
    return jax.nn.sigmoid(x)
def _layernorm(x, axis=-1, eps=1e-5):
    m = jnp.mean(x, axis=axis, keepdims=True)
    v = jnp.var(x, axis=axis, keepdims=True)
    return (x - m) / jnp.sqrt(v + eps)
def _scatter_add(tgt, idx, src, axis=0):
    return tgt.at[idx].add(src)
def _segment_sum(src, seg, n):
    return jax.ops.segment_sum(src, seg, n)
class _Rng:
    def __init__(self, key):
        self._k = key
    def _next(self):
        self._k, sub = jax.random.split(self._k)
        return sub
    def normal(self, shape):
        return jax.random.normal(self._next(), shape, dtype=jnp.bfloat16)
    def randint(self, lo, hi, shape):
        return jax.random.randint(self._next(), shape, lo, hi, dtype=jnp.int32)
    def uniform(self, shape, lo=0.0, hi=1.0):
        return jax.random.uniform(self._next(), shape, jnp.bfloat16, lo, hi)
    def permutation(self, n):
        return jax.random.permutation(self._next(), n)


kernel_name = 'concat_heads__softmax_full_mha__ssm_conv_s5__prompt'

def setup_inputs():
    _rng = _Rng(jax.random.key(int.from_bytes(__import__("os").urandom(4), "little")))
    _w = (lambda a: (lambda t: t.astype(jnp.bfloat16) if jnp.issubdtype(t.dtype, jnp.floating) else t)(jnp.asarray(a)))
    def _A_setup():
        B, S, D = 1, 2048, 512
        return {
            "x": _w((lambda *s: _rng.normal(s) * 0.2)(B, S, D)),
            "wqkv": _w((lambda *s: _rng.normal(s) * 0.2)(D, 3 * D)),
            "wo": _w((lambda *s: _rng.normal(s) * 0.05)(D, D)),
        }
    _A_in = _A_setup()

    def _B_setup():
        B, S, D = 1, 2048, 512
        P = D
        Lambda_re = -0.5 * jnp.exp((lambda *s: _rng.normal(s) * 0.4)(P))
        Lambda_im = (lambda *s: _rng.normal(s) * 0.4)(P) * 1.0
        B_re = (lambda *s: _rng.normal(s) * 0.4)(P, D) * (D ** -0.5)
        B_im = (lambda *s: _rng.normal(s) * 0.4)(P, D) * (D ** -0.5)
        C_re = (lambda *s: _rng.normal(s) * 0.4)(D, P) * (P ** -0.5)
        C_im = (lambda *s: _rng.normal(s) * 0.4)(D, P) * (P ** -0.5)
        log_dt = (lambda *s: _rng.normal(s) * 0.4)(P) * 0.3 - 2.0
        Dskip = (lambda *s: _rng.normal(s) * 0.4)(D)
        return {
            "x": _w((lambda *s: _rng.normal(s) * 0.05)(B, S, D)),
            "Lambda_re": _w(Lambda_re),
            "Lambda_im": _w(Lambda_im),
            "B_re": _w(B_re),
            "B_im": _w(B_im),
            "C_re": _w(C_re),
            "C_im": _w(C_im),
            "log_dt": _w(log_dt),
            "Dskip": _w(Dskip),
        }
    _B_in = _B_setup()

    return {
        "A_x": _A_in["x"],
        "A_wqkv": _A_in["wqkv"],
        "A_wo": _A_in["wo"],
        "B_x": _B_in["x"],
        "B_Lambda_re": _B_in["Lambda_re"],
        "B_Lambda_im": _B_in["Lambda_im"],
        "B_B_re": _B_in["B_re"],
        "B_B_im": _B_in["B_im"],
        "B_C_re": _B_in["C_re"],
        "B_C_im": _B_in["C_im"],
        "B_log_dt": _B_in["log_dt"],
        "B_Dskip": _B_in["Dskip"],
    }

def reference(A_x, A_wqkv, A_wo, B_x, B_Lambda_re, B_Lambda_im, B_B_re, B_B_im, B_C_re, B_C_im, B_log_dt, B_Dskip):
    def _A_ref(x, wqkv, wo):
        B, S, D = x.shape
        H = 32; Dh = D // H
        qkv = (lambda x, *d: x.transpose(*d))((x @ wqkv).reshape(B, S, 3, H, Dh), 2, 0, 3, 1, 4)
        q, k, v = qkv[0], qkv[1], qkv[2]
        scale = Dh ** -0.5
        scores = jnp.einsum("bhqd,bhkd->bhqk", q, k) * scale
        p = _softmax(scores, axis=-1)
        o = jnp.einsum("bhqk,bhkd->bhqd", p, v)
        return (lambda x, *d: x.transpose(*d))(o, 0, 2, 1, 3).reshape(B, S, D) @ wo

    def _B_ref(x, Lambda_re, Lambda_im, B_re, B_im, C_re, C_im, log_dt, Dskip):
        Bsz, L, H = x.shape
        Lam = Lambda_re + 1j * Lambda_im
        Bmat = B_re + 1j * B_im
        Cmat = C_re + 1j * C_im
        dt = jnp.exp(log_dt)
        Lam_bar = jnp.exp(dt * Lam)
        B_bar = ((Lam_bar - 1.0) / Lam)[:, None] * Bmat
        Bu = jnp.einsum("bld,pd->blp", x + 0j, B_bar)
        h = jnp.zeros_like(Bu[:, 0, :])
        hs = []
        for t in range(L):
            h = Lam_bar[None, :] * h + Bu[:, t, :]
            hs.append(h)
        hseq = jnp.stack(hs, 1)
        y = 2.0 * jnp.einsum("blp,dp->bld", hseq, Cmat).real + x * Dskip[None, None, :]
        return y

    a = _A_ref(A_x, A_wqkv, A_wo)
    b = _B_ref(B_x, B_Lambda_re, B_Lambda_im, B_B_re, B_B_im, B_C_re, B_C_im, B_log_dt, B_Dskip)
    return jnp.concatenate([a, b], axis=-1)
```

```python
import functools
import math

import jax
import jax.numpy as jnp
from jax import lax
from jax.experimental import pallas as pl
from jax.experimental.pallas import tpu as pltpu

S = 2048
D = 512
DH = 16
HPG = 8
NG = 4
NQ = 512
NQB = S // NQ
RB = 256
NRB = S // RB
CK = 128
NCK = S // CK
G = 32
GPC = CK // G
LEAD = 1
NT = NQ // 128
QSCALE = (DH ** -0.5) * math.log2(math.e)

F32 = jnp.float32
BF16 = jnp.bfloat16


def _nt(a, b):
    return lax.dot_general(a, b, (((1,), (1,)), ((), ())), preferred_element_type=F32)


def _tn(a, b):
    return lax.dot_general(a, b, (((0,), (0,)), ((), ())), preferred_element_type=F32)


def _nn(a, b):
    return jnp.dot(a, b, preferred_element_type=F32)


def _kernel(xa, wqkv, wo, xb, lre, lim, bre, bim, cre, cim, ldt, dsk, out,
            wqT, wvT, bcat, ccat, coef, k_all, qT_all, vT_all, oT_all,
            kc, vc, wc, s_buf, m_buf, zv, u_scr, h_scr, y_stage, a_stage, sem_y, sem_a):
    zv[...] = jnp.zeros(zv.shape, F32)
    wqT[...] = wqkv[:, 0:D].astype(F32).T.astype(BF16)
    wvT[...] = wqkv[:, 2 * D:3 * D].astype(F32).T.astype(BF16)
    bcat[0:D, :] = bre[...]
    bcat[D:2 * D, :] = bim[...]

    l_re = lre[...].astype(F32).reshape(1, D)
    l_im = lim[...].astype(F32).reshape(1, D)
    dt = jnp.exp(ldt[...].astype(F32).reshape(1, D)).astype(BF16).astype(F32)
    e_re = dt * l_re
    e_im = dt * l_im

    def apow(k):
        mag = jnp.exp(k * e_re)
        return mag * jnp.cos(k * e_im), mag * jnp.sin(k * e_im)

    a1r, a1i = apow(1.0)
    for n, k in enumerate((1.0, 2.0, 4.0, 8.0)):
        r, i = apow(k)
        coef[2 * n] = jnp.broadcast_to(r, (8, D))
        coef[2 * n + 1] = jnp.broadcast_to(i, (8, D))
    nr = a1r - 1.0
    den = l_re * l_re + l_im * l_im
    f_re = 2.0 * (nr * l_re + a1i * l_im) / den
    f_im = 2.0 * (a1i * l_re - nr * l_im) / den
    c_re = cre[...].astype(F32)
    c_im = cim[...].astype(F32)
    ccat[:, 0:D] = (c_re * f_re - c_im * f_im).astype(BF16)
    ccat[:, D:2 * D] = (-(c_re * f_im + c_im * f_re)).astype(BF16)
    dskip = dsk[...].astype(F32).reshape(1, D)

    u_scr[:, 0:8, :] = jnp.zeros((8, 8, 128), F32)
    h_scr[...] = jnp.zeros(h_scr.shape, F32)

    def y_copy(i):
        r0 = pl.multiple_of(i * RB, RB)
        return pltpu.make_async_copy(
            y_stage.at[pl.ds(r0, RB), :], out.at[pl.ds(r0, RB), pl.ds(D, D)], sem_y.at[i])

    def a_copy(qb):
        r0 = pl.multiple_of(qb * NQ, NQ)
        return pltpu.make_async_copy(
            a_stage.at[pl.ds(r0, NQ), :], out.at[pl.ds(r0, NQ), pl.ds(0, D)], sem_a.at[qb])

    def dense(i, carry):
        r0 = pl.multiple_of(i * RB, RB)
        rows = pl.ds(r0, RB)
        xb_blk = xb[rows, :]
        u = _nt(xb_blk, bcat[...])
        for c in range(8):
            u_scr[c, 8:8 + RB, :] = u[:, c * 128:(c + 1) * 128]
        xa_blk = xa[rows, :]
        kb = _nn(xa_blk, wqkv[:, D:2 * D]).astype(BF16)
        for g in range(NG):
            k_all[g, rows, :] = kb[:, g * 128:(g + 1) * 128]
        qT_all[i] = (_nt(wqT[...], xa_blk) * QSCALE).astype(BF16)
        vT_all[i] = _nt(wvT[...], xa_blk).astype(BF16)
        hs = []
        for c in range(4):
            lanes = slice(c * 128, (c + 1) * 128)
            wr = u_scr[c]
            wi = u_scr[4 + c]
            halo_r = wr[RB:RB + 8]
            halo_i = wi[RB:RB + 8]
            for n, k in enumerate((1, 2, 4)):
                ar = coef[2 * n, :, lanes]
                ai = coef[2 * n + 1, :, lanes]
                sr = pltpu.roll(wr, k, 0).reshape(RB // 8 + 1, 8, 128)
                si = pltpu.roll(wi, k, 0).reshape(RB // 8 + 1, 8, 128)
                wr3 = wr.reshape(RB // 8 + 1, 8, 128) + ar[None] * sr - ai[None] * si
                wi3 = wi.reshape(RB // 8 + 1, 8, 128) + ar[None] * si + ai[None] * sr
                wr = wr3.reshape(RB + 8, 128)
                wi = wi3.reshape(RB + 8, 128)
            ar = coef[6, :, lanes]
            ai = coef[7, :, lanes]
            hr = h_scr[c]
            hi = h_scr[4 + c]
            outr, outi = [], []
            for tl in range(RB // 8):
                w_r = wr[8 + tl * 8:16 + tl * 8]
                w_i = wi[8 + tl * 8:16 + tl * 8]
                hr, hi = w_r + ar * hr - ai * hi, w_i + ar * hi + ai * hr
                outr.append(hr)
                outi.append(hi)
            h_scr[c] = hr
            h_scr[4 + c] = hi
            u_scr[c, 0:8, :] = halo_r
            u_scr[4 + c, 0:8, :] = halo_i
            hs.append((jnp.concatenate(outr, axis=0).astype(BF16), jnp.concatenate(outi, axis=0).astype(BF16)))
        hcat = jnp.concatenate([h[0] for h in hs] + [h[1] for h in hs], axis=1)
        y = _nt(hcat, ccat[...])
        skip = (xb_blk.astype(F32) * dskip).astype(BF16).astype(F32)
        y_stage[rows, :] = y + skip
        y_copy(i).start()
        return carry

    lax.fori_loop(0, NRB, dense, 0)

    def wmat(rows16, j):
        parts = []
        if j > 0:
            parts.append(jnp.zeros((DH * j, NQ), BF16))
        parts.append(rows16)
        if j < HPG - 1:
            parts.append(jnp.zeros((DH * (HPG - 1 - j), NQ), BF16))
        return jnp.concatenate(parts, axis=0)

    def q_rows(g, qb, j):
        r = pl.ds(pl.multiple_of(g * 128 + j * DH, DH), DH)
        return jnp.concatenate([qT_all[2 * qb, r, :], qT_all[2 * qb + 1, r, :]], axis=1)

    s0 = _nn(k_all[0], wmat(q_rows(0, 0, 0), 0))
    s_buf[0] = s0
    m_buf[...] = jnp.max(s0, axis=0, keepdims=True)

    def attn(t, carry):
        g = t // NQB
        qb = t % NQB
        tn = jnp.minimum(t + 1, NG * NQB - 1)
        gn = tn // NQB
        qbn = tn % NQB

        @pl.when(qb == 0)
        def _():
            kc[...] = k_all[g]
            gr = pl.ds(pl.multiple_of(g * 128, 128), 128)
            for b in range(NRB):
                vc[:, b * RB:(b + 1) * RB] = vT_all[b, gr, :]

        gr = pl.ds(pl.multiple_of(g * 128, 128), 128)
        wc[:, 0:RB] = qT_all[2 * qb, gr, :]
        wc[:, RB:2 * RB] = qT_all[2 * qb + 1, gr, :]

        z = zv[...]
        NJ = HPG * NCK
        ng = NJ * GPC
        st = {}
        ps = {}

        def adot(J):
            a = J // NCK + 1
            c = J % NCK
            if a < HPG:
                return _nn(kc[c * CK:(c + 1) * CK, :], wmat(wc[a * DH:(a + 1) * DH, :], a))
            return _nn(k_all[gn, c * CK:(c + 1) * CK, :], wmat(q_rows(gn, qbn, 0), 0))

        def s2_group(g2, gate):
            J2 = g2 // GPC
            r = g2 % GPC
            j = J2 // NCK
            c = J2 % NCK
            if c == 0 and r == 0:
                st['m'] = jnp.broadcast_to(st['mfin'], (8, NQ))
                st['l'] = jnp.zeros((8, NQ), F32)
                st[('o', j)] = jnp.zeros((DH, NQ), F32)
            x = s_buf[j % 2, c * CK + r * G: c * CK + (r + 1) * G, :].reshape(G // 8, 8, NQ)
            if gate is not None:
                mg = st['m'] + jnp.concatenate([gate * z] * NT, axis=1)
            else:
                mg = st['m']
            p = jnp.exp2(x - mg[None])
            st['l'] = st['l'] + jnp.sum(p, axis=0)
            ps[g2] = p.reshape(G, NQ)
            if c == NCK - 1 and r == GPC - 1:
                st[('lfin', j)] = st['l']

        def pv(J2):
            j = J2 // NCK
            c = J2 % NCK
            pb = jnp.concatenate([ps.pop(J2 * GPC + r) for r in range(GPC)], axis=0).astype(BF16)
            st[('o', j)] = st[('o', j)] + _nn(vc[j * DH:(j + 1) * DH, c * CK:(c + 1) * CK], pb)
            if c == NCK - 1:
                o = st.pop(('o', j)) / jnp.sum(st.pop(('lfin', j)), axis=0, keepdims=True)
                orow = pl.ds(pl.multiple_of(g * 128 + j * DH, DH), DH)
                oT_all[qb, orow, :] = o.astype(BF16)

        def can2(g2, J, r):
            j = g2 // GPC // NCK
            return j == 0 or (J, r) >= (j * NCK - 1, GPC - 1)

        st['mfin'] = m_buf[...]
        s_next = adot(0)
        done2 = 0
        for _ in range(LEAD):
            s2_group(done2, None)
            done2 += 1
        pv_done = 0
        for J in range(NJ):
            a = J // NCK + 1
            c = J % NCK
            s = s_next
            if J + 1 < NJ:
                s_next = adot(J + 1)
            if c == 0:
                mx = jnp.full((8, NQ), -jnp.inf, F32)
            for r in range(GPC):
                sg = s[r * G:(r + 1) * G]
                s_buf[a % 2, c * CK + r * G: c * CK + (r + 1) * G, :] = sg
                mx = jnp.maximum(mx, jnp.max(sg.reshape(G // 8, 8, NQ), axis=0))
                if c == NCK - 1 and r == GPC - 1:
                    st['mfin'] = jnp.max(mx, axis=0, keepdims=True)
                target = min(ng, J * GPC + r + 1 + LEAD)
                while done2 < target and can2(done2, J, r):
                    s2_group(done2, sg[0:8, 0:128])
                    done2 += 1
            while pv_done < NJ and (pv_done + 1) * GPC <= done2 and pv_done <= J:
                pv(pv_done)
                pv_done += 1
        while pv_done < NJ:
            pv(pv_done)
            pv_done += 1
        m_buf[...] = st['mfin']

        @pl.when(g == NG - 1)
        def _():
            r0 = pl.multiple_of(qb * NQ, NQ)
            a_stage[pl.ds(r0, NQ), :] = _tn(oT_all[qb], wo[...])
            a_copy(qb).start()

        return carry

    lax.fori_loop(0, NG * NQB, attn, 0)

    for i in range(NRB):
        y_copy(i).wait()
    for qb in range(NQB):
        a_copy(qb).wait()


@jax.jit
def pallas_concat_heads__softmax_full_mha__ssm_conv_s5__prompt_kernel(A_x, A_wqkv, A_wo, B_x, B_Lambda_re, B_Lambda_im, B_B_re, B_B_im, B_C_re, B_C_im, B_log_dt, B_Dskip):
    xa = A_x.reshape(S, D)
    xb = B_x.reshape(S, D)
    vm = pl.BlockSpec(memory_space=pltpu.VMEM)
    out = pl.pallas_call(
        _kernel,
        out_shape=jax.ShapeDtypeStruct((S, 2 * D), F32),
        in_specs=[vm] * 12,
        out_specs=pl.BlockSpec(memory_space=pl.ANY),
        scratch_shapes=[
            pltpu.VMEM((D, D), BF16),
            pltpu.VMEM((D, D), BF16),
            pltpu.VMEM((2 * D, D), BF16),
            pltpu.VMEM((D, 2 * D), BF16),
            pltpu.VMEM((8, 8, D), F32),
            pltpu.VMEM((NG, S, 128), BF16),
            pltpu.VMEM((NRB, D, RB), BF16),
            pltpu.VMEM((NRB, D, RB), BF16),
            pltpu.VMEM((NQB, D, NQ), BF16),
            pltpu.VMEM((S, 128), BF16),
            pltpu.VMEM((128, S), BF16),
            pltpu.VMEM((128, NQ), BF16),
            pltpu.VMEM((2, S, NQ), F32),
            pltpu.VMEM((1, NQ), F32),
            pltpu.VMEM((8, 128), F32),
            pltpu.VMEM((8, RB + 8, 128), F32),
            pltpu.VMEM((8, 8, 128), F32),
            pltpu.VMEM((S, D), F32),
            pltpu.VMEM((S, D), F32),
            pltpu.SemaphoreType.DMA((NRB,)),
            pltpu.SemaphoreType.DMA((NQB,)),
        ],
        compiler_params=pltpu.CompilerParams(vmem_limit_bytes=100 * 2 ** 20),
        name="fused_mha_s5",
    )(xa, A_wqkv, A_wo, xb, B_Lambda_re, B_Lambda_im, B_B_re, B_B_im, B_C_re, B_C_im, B_log_dt, B_Dskip)
    return out.reshape(1, S, 2 * D)
```

```python
import math

import jax
import jax.numpy as jnp
from jax import lax
from jax.experimental import pallas as pl
from jax.experimental.pallas import tpu as pltpu

S = 2048
D = 512
DH = 16
HPG = 8
NG = 4
NQ = 512
NQB = S // NQ
NB = NG * NQB
RB = 256
NRB = S // RB
SB = S // NB
CK = 128
NCK = S // CK
NJ = HPG * NCK
G = 32
GPC = CK // G
LEAD = 1
NT = NQ // 128
SCAN0 = 4
SCANSTEP = 7
QSCALE = (DH ** -0.5) * math.log2(math.e)

F32 = jnp.float32
BF16 = jnp.bfloat16
I32 = jnp.int32


def _nt(a, b):
    return lax.dot_general(a, b, (((1,), (1,)), ((), ())), preferred_element_type=F32)


def _tn(a, b):
    return lax.dot_general(a, b, (((0,), (0,)), ((), ())), preferred_element_type=F32)


def _nn(a, b):
    return jnp.dot(a, b, preferred_element_type=F32)


def _kernel(xa_h, wqkv_h, wo_h, xb_h, lre, lim, bre_h, bim_h, cre_h, cim_h, ldt, dsk, out,
            xa, wqkv, wo, xb, bcat, ccat, coef, k_all, qT_all, vT_all, oT_prev, oT_cur,
            kc, vc, vprev, wc, s_buf, m_buf, zv, u_scr, h_scr, y_stage, a_stage,
            sem_w, sem_x, sem_y, sem_a):
    def x_copy(i):
        r = pl.ds(pl.multiple_of(i * RB, RB), RB)
        return pltpu.make_async_copy(xa_h.at[r, :], xa.at[r, :], sem_x.at[i])

    def wq_copy(n):
        c = pl.ds(n * D, D)
        return pltpu.make_async_copy(wqkv_h.at[:, c], wqkv.at[:, c], sem_w.at[n])

    w_copies = [
        pltpu.make_async_copy(bre_h, bcat.at[pl.ds(0, D), :], sem_w.at[3]),
        pltpu.make_async_copy(bim_h, bcat.at[pl.ds(D, D), :], sem_w.at[4]),
        pltpu.make_async_copy(xb_h, xb, sem_w.at[5]),
        pltpu.make_async_copy(cre_h, ccat.at[:, pl.ds(0, D)], sem_w.at[6]),
        pltpu.make_async_copy(cim_h, ccat.at[:, pl.ds(D, D)], sem_w.at[7]),
        pltpu.make_async_copy(wo_h, wo, sem_w.at[8]),
    ]
    x_copy(0).start()
    wq_copy(0).start()
    wq_copy(2).start()
    wq_copy(1).start()
    x_copy(1).start()

    zv[...] = jnp.zeros(zv.shape, I32)
    oT_prev[...] = jnp.zeros((128, NQ), BF16)
    vprev[...] = jnp.zeros(vprev.shape, BF16)
    m_buf[...] = jnp.zeros(m_buf.shape, F32)
    u_scr[:, 0:8, :] = jnp.zeros((8, 8, 128), F32)
    h_scr[...] = jnp.zeros(h_scr.shape, F32)

    l_re = lre[...].astype(F32).reshape(1, D)
    l_im = lim[...].astype(F32).reshape(1, D)
    dt = jnp.exp(ldt[...].astype(F32).reshape(1, D)).astype(BF16).astype(F32)
    e_re = dt * l_re
    e_im = dt * l_im

    def apow(k):
        mag = jnp.exp(k * e_re)
        return mag * jnp.cos(k * e_im), mag * jnp.sin(k * e_im)

    a1r, a1i = apow(1.0)
    for n, k in enumerate((1.0, 2.0, 4.0, 8.0)):
        r, i = apow(k)
        coef[2 * n] = jnp.broadcast_to(r, (8, D))
        coef[2 * n + 1] = jnp.broadcast_to(i, (8, D))
    nr = a1r - 1.0
    den = l_re * l_re + l_im * l_im
    coef[8] = jnp.broadcast_to(2.0 * (nr * l_re + a1i * l_im) / den, (8, D))
    coef[9] = jnp.broadcast_to(2.0 * (a1i * l_re - nr * l_im) / den, (8, D))
    coef[10] = jnp.broadcast_to(dsk[...].astype(F32).reshape(1, D), (8, D))

    def proj_q(i, xa_blk):
        qT_all[i] = (_nn(xa_blk, wqkv[:, 0:D]) * QSCALE).astype(BF16).T

    def proj_v(i, xa_blk):
        vT_all[i] = _nn(xa_blk, wqkv[:, 2 * D:3 * D]).astype(BF16).T

    def proj_k(rows, xa_blk):
        kb = _nn(xa_blk, wqkv[:, D:2 * D]).astype(BF16)
        for g in range(NG):
            k_all[g, rows, :] = kb[:, g * 128:(g + 1) * 128]
        a_stage[rows, :] = jnp.zeros((RB, D), F32)
        s_buf[1, rows, :] = jnp.zeros((RB, NQ), F32)

    x_copy(0).wait()
    wq_copy(0).wait()
    proj_q(0, xa[0:RB, :])
    wq_copy(2).wait()
    for i in range(2, NRB):
        x_copy(i).start()
    proj_v(0, xa[0:RB, :])
    wq_copy(1).wait()
    for cp in w_copies:
        cp.start()
    proj_k(pl.ds(0, RB), xa[0:RB, :])

    def proj(i, carry):
        x_copy(i).wait()
        rows = pl.ds(pl.multiple_of(i * RB, RB), RB)
        xa_blk = xa[rows, :]
        proj_q(i, xa_blk)
        proj_v(i, xa_blk)
        proj_k(rows, xa_blk)
        return carry

    lax.fori_loop(1, NRB, proj, 0)
    for cp in w_copies:
        cp.wait()

    def wmat(j):
        parts = []
        if j > 0:
            parts.append(jnp.zeros((DH * j, NQ), BF16))
        parts.append(wc[j * DH:(j + 1) * DH, :])
        if j < HPG - 1:
            parts.append(jnp.zeros((DH * (HPG - 1 - j), NQ), BF16))
        return jnp.concatenate(parts, axis=0)

    def y_copy(t):
        r = pl.ds(pl.multiple_of(t * SB, SB), SB)
        return pltpu.make_async_copy(y_stage.at[r, :], out.at[r, pl.ds(D, D)], sem_y.at[t])

    def a_copy(qb_):
        r = pl.ds(pl.multiple_of(qb_ * NQ, NQ), NQ)
        return pltpu.make_async_copy(a_stage.at[r, :], out.at[r, pl.ds(0, D)], sem_a.at[qb_])

    rowid = lax.broadcasted_iota(I32, (8, 128), 0)

    class Scan:
        def __init__(self):
            self.prev = {}
            self.h = [(h_scr[c], h_scr[4 + c]) for c in range(4)]
            self.out = []

        def _fir(self, c, ur, ui, halo):
            lanes = slice(c * 128, (c + 1) * 128)
            wr, wi = ur, ui
            for n, k in enumerate((1, 2, 4)):
                rr = pltpu.roll(wr, k, 0)
                ri = pltpu.roll(wi, k, 0)
                if halo:
                    sr, si = rr, ri
                else:
                    pr, pi = self.prev[(c, n)]
                    sr = jnp.where(rowid < k, pr, rr)
                    si = jnp.where(rowid < k, pi, ri)
                self.prev[(c, n)] = (rr, ri)
                if halo and n == 2:
                    break
                ar = coef[2 * n, :, lanes]
                ai = coef[2 * n + 1, :, lanes]
                wr, wi = wr + ar * sr - ai * si, wi + ar * si + ai * sr
            return wr, wi

        def halo(self):
            for c in range(4):
                self._fir(c, u_scr[c, 0:8, :], u_scr[4 + c, 0:8, :], True)

        def step(self, tile, gate):
            rows = slice(8 + tile * 8, 16 + tile * 8)
            res = []
            for c in range(4):
                lanes = slice(c * 128, (c + 1) * 128)
                wr, wi = self._fir(c, u_scr[c, rows, :] + gate, u_scr[4 + c, rows, :] + gate, False)
                ar = coef[6, :, lanes]
                ai = coef[7, :, lanes]
                hr, hi = self.h[c]
                hr, hi = wr + ar * hr - ai * hi, wi + ar * hi + ai * hr
                self.h[c] = (hr, hi)
                fr = coef[8, :, lanes]
                fi = coef[9, :, lanes]
                res.append((fr * hr - fi * hi, -(fr * hi + fi * hr)))
            self.out.append(jnp.concatenate([r[0] for r in res] + [r[1] for r in res], axis=1))

        def finish(self):
            for c in range(4):
                h_scr[c] = self.h[c][0]
                h_scr[4 + c] = self.h[c][1]
            for c in range(8):
                u_scr[c, 0:8, :] = u_scr[c, SB:SB + 8, :]
            return jnp.concatenate(self.out, axis=0).astype(BF16)

    class Stage2:
        def __init__(self, store_o):
            self.st = {}
            self.ps = {}
            self.store_o = store_o

        def group(self, g2, gate):
            st = self.st
            J2 = g2 // GPC
            r = GPC - 1 - g2 % GPC
            j2 = J2 // NCK
            c = J2 % NCK
            if c == 0 and g2 % GPC == 0:
                st['m'] = jnp.broadcast_to(st['mfin'], (8, NQ))
                st['l'] = jnp.zeros((8, NQ), F32)
                st[('o', j2)] = jnp.zeros((DH, NQ), F32)
            x = s_buf[(j2 + 1) % 2, c * CK + r * G: c * CK + (r + 1) * G, :].reshape(G // 8, 8, NQ)
            if gate is not None:
                st['m'] = st['m'] + jnp.concatenate([gate] * NT, axis=1)
            p = jnp.exp2(x - st['m'][None])
            st['l'] = st['l'] + jnp.sum(p, axis=0)
            self.ps[(J2, r)] = p.reshape(G, NQ)
            if c == NCK - 1 and r == 0:
                st[('lfin', j2)] = st['l']

        def pv(self, J2):
            st = self.st
            j2 = J2 // NCK
            c = J2 % NCK
            pb = jnp.concatenate([self.ps.pop((J2, r)) for r in range(GPC)], axis=0).astype(BF16)
            if j2 == 0:
                vt = vprev[:, c * CK:(c + 1) * CK]
            else:
                vt = vc[(j2 - 1) * DH:j2 * DH, c * CK:(c + 1) * CK]
            st[('o', j2)] = st[('o', j2)] + _nn(vt, pb)
            if c == NCK - 1:
                o = st.pop(('o', j2)) / jnp.sum(st.pop(('lfin', j2)), axis=0, keepdims=True)
                self.store_o(j2, o.astype(BF16))

    def attn(t, carry):
        g = t // NQB
        qbi = t % NQB
        tp = jnp.maximum(t - 1, 0)

        @pl.when(qbi == 0)
        def _():
            kc[...] = k_all[g]
            gr = pl.ds(pl.multiple_of(g * 128, 128), 128)
            for b in range(NRB):
                vc[:, b * RB:(b + 1) * RB] = vT_all[b, gr, :]

        gr = pl.ds(pl.multiple_of(g * 128, 128), 128)
        wc[:, 0:RB] = qT_all[2 * qbi, gr, :]
        wc[:, RB:2 * RB] = qT_all[2 * qbi + 1, gr, :]

        srows = pl.ds(pl.multiple_of(t * SB, SB), SB)
        xb_blk = xb[srows, :]
        u = _nt(xb_blk, bcat[...])
        for c in range(8):
            u_scr[c, 8:8 + SB, :] = u[:, c * 128:(c + 1) * 128]
        scan = Scan()
        scan.halo()

        zi = zv[...]

        def zgate(x):
            return lax.bitcast_convert_type(lax.bitcast_convert_type(x, I32) & zi, F32)

        def store_o(j2, o):
            if j2 == 0:
                oT_prev[(HPG - 1) * DH:HPG * DH, :] = o
            else:
                oT_cur[(j2 - 1) * DH:j2 * DH, :] = o

        s2 = Stage2(store_o)
        ng = NJ * GPC

        def adot(J):
            c = J % NCK
            return _nn(kc[c * CK:(c + 1) * CK, :], wmat(J // NCK))

        def can2(g2, J, r):
            j2 = g2 // GPC // NCK
            return j2 == 0 or (J, r) >= (j2 * NCK - 1, GPC - 1)

        s2.st['mfin'] = m_buf[...]
        s_next = adot(0)
        done2 = 0
        for _ in range(LEAD):
            s2.group(done2, None)
            done2 += 1
        pv_done = 0
        for J in range(NJ):
            a = J // NCK
            c = J % NCK
            s = s_next
            if J + 1 < NJ:
                s_next = adot(J + 1)
            if c == 0:
                mx = jnp.full((8, NQ), -jnp.inf, F32)
            for r in range(GPC):
                sg = s[r * G:(r + 1) * G]
                s_buf[a % 2, c * CK + r * G: c * CK + (r + 1) * G, :] = sg
                mx = jnp.maximum(mx, jnp.max(sg.reshape(G // 8, 8, NQ), axis=0))
                if c == NCK - 1 and r == GPC - 1:
                    s2.st['mfin'] = jnp.max(mx, axis=0, keepdims=True)
                gate = zgate(sg[0:8, 0:128])
                if r == 0 and J >= SCAN0 and (J - SCAN0) % SCANSTEP == 0 and (J - SCAN0) // SCANSTEP < SB // 8:
                    scan.step((J - SCAN0) // SCANSTEP, gate)
                target = min(ng, J * GPC + r + 1 + LEAD)
                while done2 < target and can2(done2, J, r):
                    s2.group(done2, gate)
                    done2 += 1
            last = NJ - 1 if J == NJ - 1 else NJ
            while pv_done < last and (pv_done + 1) * GPC <= done2 and pv_done <= J:
                s2.pv(pv_done)
                pv_done += 1
        y = _nt(scan.finish(), ccat[...])
        skip = (xb_blk.astype(F32) * coef[10, 0:1, :]).astype(BF16).astype(F32)
        y_stage[srows, :] = y + skip
        while pv_done < NJ:
            s2.pv(pv_done)
            pv_done += 1
        m_buf[...] = s2.st['mfin']
        vprev[...] = vc[(HPG - 1) * DH:HPG * DH, :]
        p_rows = pl.ds(pl.multiple_of((tp % NQB) * NQ, NQ), NQ)
        p_wo = wo[pl.ds(pl.multiple_of((tp // NQB) * 128, 128), 128), :]
        a_stage[p_rows, :] = a_stage[p_rows, :] + _tn(oT_prev[...], p_wo)
        oT_prev[0:(HPG - 1) * DH, :] = oT_cur[0:(HPG - 1) * DH, :]
        y_copy(t).start()

        @pl.when(t > (NG - 1) * NQB)
        def _():
            a_copy(tp % NQB).start()

        return carry

    lax.fori_loop(0, NB, attn, 0)

    def store_last(j2, o):
        oT_prev[(HPG - 1) * DH:HPG * DH, :] = o

    s2 = Stage2(store_last)
    s2.st['mfin'] = m_buf[...]
    for J2 in range(NCK):
        for r in range(GPC):
            s2.group(J2 * GPC + r, None)
        s2.pv(J2)
    o_last = oT_prev[...]
    wo_last = wo[(NG - 1) * 128:NG * 128, :]
    tail = []
    for n in range(4):
        r0 = (NQB - 1) * NQ + n * 128
        a_stage[r0:r0 + 128, :] = a_stage[r0:r0 + 128, :] + _tn(o_last[:, n * 128:(n + 1) * 128], wo_last)
        cp = pltpu.make_async_copy(a_stage.at[pl.ds(r0, 128), :], out.at[pl.ds(r0, 128), pl.ds(0, D)], sem_a.at[NQB - 1 + n])
        cp.start()
        tail.append(cp)

    for t in range(NB):
        y_copy(t).wait()
    for qb_ in range(NQB - 1):
        a_copy(qb_).wait()
    for cp in tail:
        cp.wait()


@jax.jit
def pallas_concat_heads__softmax_full_mha__ssm_conv_s5__prompt_kernel(A_x, A_wqkv, A_wo, B_x, B_Lambda_re, B_Lambda_im, B_B_re, B_B_im, B_C_re, B_C_im, B_log_dt, B_Dskip):
    xa = A_x.reshape(S, D)
    xb = B_x.reshape(S, D)
    vm = pl.BlockSpec(memory_space=pltpu.VMEM)
    hbm = pl.BlockSpec(memory_space=pl.ANY)
    out = pl.pallas_call(
        _kernel,
        out_shape=jax.ShapeDtypeStruct((S, 2 * D), F32),
        in_specs=[hbm, hbm, hbm, hbm, vm, vm, hbm, hbm, hbm, hbm, vm, vm],
        out_specs=hbm,
        scratch_shapes=[
            pltpu.VMEM((S, D), BF16),
            pltpu.VMEM((D, 3 * D), BF16),
            pltpu.VMEM((D, D), BF16),
            pltpu.VMEM((S, D), BF16),
            pltpu.VMEM((2 * D, D), BF16),
            pltpu.VMEM((D, 2 * D), BF16),
            pltpu.VMEM((11, 8, D), F32),
            pltpu.VMEM((NG, S, 128), BF16),
            pltpu.VMEM((NRB, D, RB), BF16),
            pltpu.VMEM((NRB, D, RB), BF16),
            pltpu.VMEM((128, NQ), BF16),
            pltpu.VMEM((128, NQ), BF16),
            pltpu.VMEM((S, 128), BF16),
            pltpu.VMEM((128, S), BF16),
            pltpu.VMEM((DH, S), BF16),
            pltpu.VMEM((128, NQ), BF16),
            pltpu.VMEM((2, S, NQ), F32),
            pltpu.VMEM((1, NQ), F32),
            pltpu.VMEM((8, 128), I32),
            pltpu.VMEM((8, SB + 8, 128), F32),
            pltpu.VMEM((8, 8, 128), F32),
            pltpu.VMEM((S, D), F32),
            pltpu.VMEM((S, D), F32),
            pltpu.SemaphoreType.DMA((9,)),
            pltpu.SemaphoreType.DMA((NRB,)),
            pltpu.SemaphoreType.DMA((NB,)),
            pltpu.SemaphoreType.DMA((NQB + 3,)),
        ],
        compiler_params=pltpu.CompilerParams(vmem_limit_bytes=100 * 2 ** 20),
        name="fused_mha_s5",
    )(xa, A_wqkv, A_wo, xb, B_Lambda_re, B_Lambda_im, B_B_re, B_B_im, B_C_re, B_C_im, B_log_dt, B_Dskip)
    return out.reshape(1, S, 2 * D)
```

```python
import math

import jax
import jax.numpy as jnp
from jax import lax
from jax.experimental import pallas as pl
from jax.experimental.pallas import tpu as pltpu

S = 2048
D = 512
DH = 16
HPG = 8
NG = 4
NQ = 512
NQB = S // NQ
NB = NG * NQB
RB = 256
NRB = S // RB
SB = S // NB
CK = 128
NCK = S // CK
NJ = HPG * NCK
G = 32
GPC = CK // G
LEAD = 1
NT = NQ // 128
SCAN0 = 8
SCANSTEP = 7
QSCALE = (DH ** -0.5) * math.log2(math.e)

F32 = jnp.float32
BF16 = jnp.bfloat16
I32 = jnp.int32


def _nt(a, b):
    return lax.dot_general(a, b, (((1,), (1,)), ((), ())), preferred_element_type=F32)


def _tn(a, b):
    return lax.dot_general(a, b, (((0,), (0,)), ((), ())), preferred_element_type=F32)


def _nn(a, b):
    return jnp.dot(a, b, preferred_element_type=F32)


def _kernel(xa_h, wqkv_h, wo_h, xb_h, lre, lim, bre_h, bim_h, cre_h, cim_h, ldt, dsk, out,
            xa, wqkv, wo, xb, bcat, ccat, coef, k_all, qT_all, vT_all, oT_prev, oT_cur,
            kc, vc, vprev, wc, s_buf, m_buf, zv, u_scr, h_scr, y_stage, a_stage,
            sem_w, sem_x, sem_y, sem_a):
    def x_copy(i):
        r = pl.ds(pl.multiple_of(i * RB, RB), RB)
        return pltpu.make_async_copy(xa_h.at[r, :], xa.at[r, :], sem_x.at[i])

    def wq_copy(n):
        c = pl.ds(n * D, D)
        return pltpu.make_async_copy(wqkv_h.at[:, c], wqkv.at[:, c], sem_w.at[n])

    w_copies = [
        pltpu.make_async_copy(bre_h, bcat.at[pl.ds(0, D), :], sem_w.at[3]),
        pltpu.make_async_copy(bim_h, bcat.at[pl.ds(D, D), :], sem_w.at[4]),
        pltpu.make_async_copy(xb_h, xb, sem_w.at[5]),
        pltpu.make_async_copy(cre_h, ccat.at[:, pl.ds(0, D)], sem_w.at[6]),
        pltpu.make_async_copy(cim_h, ccat.at[:, pl.ds(D, D)], sem_w.at[7]),
        pltpu.make_async_copy(wo_h, wo, sem_w.at[8]),
    ]
    x_copy(0).start()
    wq_copy(0).start()
    wq_copy(2).start()
    wq_copy(1).start()
    x_copy(1).start()

    zv[...] = jnp.zeros(zv.shape, I32)
    oT_prev[...] = jnp.zeros((128, NQ), BF16)
    a_stage[...] = jnp.zeros(a_stage.shape, F32)
    u_scr[:, 0:8, :] = jnp.zeros((8, 8, 128), F32)
    h_scr[...] = jnp.zeros(h_scr.shape, F32)

    l_re = lre[...].astype(F32).reshape(1, D)
    l_im = lim[...].astype(F32).reshape(1, D)
    dt = jnp.exp(ldt[...].astype(F32).reshape(1, D)).astype(BF16).astype(F32)
    e_re = dt * l_re
    e_im = dt * l_im

    def apow(k):
        mag = jnp.exp(k * e_re)
        return mag * jnp.cos(k * e_im), mag * jnp.sin(k * e_im)

    a1r, a1i = apow(1.0)
    for n, k in enumerate((1.0, 2.0, 4.0, 8.0)):
        r, i = apow(k)
        coef[2 * n] = jnp.broadcast_to(r, (8, D))
        coef[2 * n + 1] = jnp.broadcast_to(i, (8, D))
    nr = a1r - 1.0
    den = l_re * l_re + l_im * l_im
    coef[8] = jnp.broadcast_to(2.0 * (nr * l_re + a1i * l_im) / den, (8, D))
    coef[9] = jnp.broadcast_to(2.0 * (a1i * l_re - nr * l_im) / den, (8, D))
    coef[10] = jnp.broadcast_to(dsk[...].astype(F32).reshape(1, D), (8, D))

    def proj_q(i, xa_blk):
        qT_all[i] = (_nn(xa_blk, wqkv[:, 0:D]) * QSCALE).astype(BF16).T

    def proj_v(i, xa_blk):
        vT_all[i] = _nn(xa_blk, wqkv[:, 2 * D:3 * D]).astype(BF16).T

    def proj_k(rows, xa_blk):
        kb = _nn(xa_blk, wqkv[:, D:2 * D]).astype(BF16)
        for g in range(NG):
            k_all[g, rows, :] = kb[:, g * 128:(g + 1) * 128]

    x_copy(0).wait()
    wq_copy(0).wait()
    proj_q(0, xa[0:RB, :])
    wq_copy(2).wait()
    for i in range(2, NRB):
        x_copy(i).start()
    proj_v(0, xa[0:RB, :])
    wq_copy(1).wait()
    for cp in w_copies:
        cp.start()
    proj_k(pl.ds(0, RB), xa[0:RB, :])

    def proj(i, carry):
        x_copy(i).wait()
        rows = pl.ds(pl.multiple_of(i * RB, RB), RB)
        xa_blk = xa[rows, :]
        proj_q(i, xa_blk)
        proj_v(i, xa_blk)
        proj_k(rows, xa_blk)
        return carry

    lax.fori_loop(1, NRB, proj, 0)
    for cp in w_copies:
        cp.wait()

    def wmat(j):
        parts = []
        if j > 0:
            parts.append(jnp.zeros((DH * j, NQ), BF16))
        parts.append(wc[j * DH:(j + 1) * DH, :])
        if j < HPG - 1:
            parts.append(jnp.zeros((DH * (HPG - 1 - j), NQ), BF16))
        return jnp.concatenate(parts, axis=0)

    def y_copy(t):
        r = pl.ds(pl.multiple_of(t * SB, SB), SB)
        return pltpu.make_async_copy(y_stage.at[r, :], out.at[r, pl.ds(D, D)], sem_y.at[t])

    def a_copy(qb_):
        r = pl.ds(pl.multiple_of(qb_ * NQ, NQ), NQ)
        return pltpu.make_async_copy(a_stage.at[r, :], out.at[r, pl.ds(0, D)], sem_a.at[qb_])

    rowid = lax.broadcasted_iota(I32, (8, 128), 0)

    class Scan:
        def __init__(self):
            self.prev = {}
            self.h = [(h_scr[c], h_scr[4 + c]) for c in range(4)]
            self.out = []

        def _fir(self, c, ur, ui, halo):
            lanes = slice(c * 128, (c + 1) * 128)
            wr, wi = ur, ui
            for n, k in enumerate((1, 2, 4)):
                rr = pltpu.roll(wr, k, 0)
                ri = pltpu.roll(wi, k, 0)
                if halo:
                    sr, si = rr, ri
                else:
                    pr, pi = self.prev[(c, n)]
                    sr = jnp.where(rowid < k, pr, rr)
                    si = jnp.where(rowid < k, pi, ri)
                self.prev[(c, n)] = (rr, ri)
                if halo and n == 2:
                    break
                ar = coef[2 * n, :, lanes]
                ai = coef[2 * n + 1, :, lanes]
                wr, wi = wr + ar * sr - ai * si, wi + ar * si + ai * sr
            return wr, wi

        def halo(self):
            for c in range(4):
                self._fir(c, u_scr[c, 0:8, :], u_scr[4 + c, 0:8, :], True)

        def step(self, tile, gate):
            rows = slice(8 + tile * 8, 16 + tile * 8)
            res = []
            for c in range(4):
                lanes = slice(c * 128, (c + 1) * 128)
                wr, wi = self._fir(c, u_scr[c, rows, :] + gate, u_scr[4 + c, rows, :] + gate, False)
                ar = coef[6, :, lanes]
                ai = coef[7, :, lanes]
                hr, hi = self.h[c]
                hr, hi = wr + ar * hr - ai * hi, wi + ar * hi + ai * hr
                self.h[c] = (hr, hi)
                fr = coef[8, :, lanes]
                fi = coef[9, :, lanes]
                res.append((fr * hr - fi * hi, -(fr * hi + fi * hr)))
            self.out.append(jnp.concatenate([r[0] for r in res] + [r[1] for r in res], axis=1))

        def finish(self):
            for c in range(4):
                h_scr[c] = self.h[c][0]
                h_scr[4 + c] = self.h[c][1]
            for c in range(8):
                u_scr[c, 0:8, :] = u_scr[c, SB:SB + 8, :]
            return jnp.concatenate(self.out, axis=0).astype(BF16)

    class Stage2:
        def __init__(self, store_o):
            self.st = {}
            self.ps = {}
            self.store_o = store_o

        def group(self, g2, gate):
            st = self.st
            J2 = g2 // GPC
            r = GPC - 1 - g2 % GPC
            j2 = J2 // NCK
            c = J2 % NCK
            if c == 0 and g2 % GPC == 0:
                st['m'] = jnp.broadcast_to(st['mfin'], (8, NQ))
                st['l'] = jnp.zeros((8, NQ), F32)
                st[('o', j2)] = jnp.zeros((DH, NQ), F32)
            x = s_buf[(j2 + 1) % 2, c * CK + r * G: c * CK + (r + 1) * G, :].reshape(G // 8, 8, NQ)
            if gate is not None:
                st['m'] = st['m'] + jnp.concatenate([gate] * NT, axis=1)
            p = jnp.exp2(x - st['m'][None])
            st['l'] = st['l'] + jnp.sum(p, axis=0)
            self.ps[(J2, r)] = p.reshape(G, NQ)
            if c == NCK - 1 and r == 0:
                st[('lfin', j2)] = st['l']

        def pv(self, J2):
            st = self.st
            j2 = J2 // NCK
            c = J2 % NCK
            pb = jnp.concatenate([self.ps.pop((J2, r)) for r in range(GPC)], axis=0).astype(BF16)
            if j2 == 0:
                vt = vprev[:, c * CK:(c + 1) * CK]
            else:
                vt = vc[(j2 - 1) * DH:j2 * DH, c * CK:(c + 1) * CK]
            st[('o', j2)] = st[('o', j2)] + _nn(vt, pb)
            if c == NCK - 1:
                o = st.pop(('o', j2)) / jnp.sum(st.pop(('lfin', j2)), axis=0, keepdims=True)
                self.store_o(j2, o.astype(BF16))

    def attn(t, carry):
        g = t // NQB
        qbi = t % NQB
        tp = jnp.maximum(t - 1, 0)

        @pl.when(qbi == 0)
        def _():
            kc[...] = k_all[g]
            gr = pl.ds(pl.multiple_of(g * 128, 128), 128)
            for b in range(NRB):
                vc[:, b * RB:(b + 1) * RB] = vT_all[b, gr, :]

        gr = pl.ds(pl.multiple_of(g * 128, 128), 128)
        wc[:, 0:RB] = qT_all[2 * qbi, gr, :]
        wc[:, RB:2 * RB] = qT_all[2 * qbi + 1, gr, :]

        srows = pl.ds(pl.multiple_of(t * SB, SB), SB)
        xb_blk = xb[srows, :]
        u = _nt(xb_blk, bcat[...])
        for c in range(8):
            u_scr[c, 8:8 + SB, :] = u[:, c * 128:(c + 1) * 128]
        scan = Scan()
        scan.halo()

        zi = zv[...]

        def zgate(x):
            return lax.bitcast_convert_type(lax.bitcast_convert_type(x, I32) & zi, F32)

        def store_o(j2, o):
            if j2 == 0:
                oT_prev[(HPG - 1) * DH:HPG * DH, :] = jnp.where(t > 0, o, jnp.zeros_like(o))
            else:
                oT_cur[(j2 - 1) * DH:j2 * DH, :] = o

        s2 = Stage2(store_o)
        ng = NJ * GPC

        def adot(J):
            c = J % NCK
            return _nn(kc[c * CK:(c + 1) * CK, :], wmat(J // NCK))

        def can2(g2, J, r):
            j2 = g2 // GPC // NCK
            return j2 == 0 or (J, r) >= (j2 * NCK - 1, GPC - 1)

        s2.st['mfin'] = m_buf[...]
        s_next = adot(0)
        done2 = 0
        for _ in range(LEAD):
            s2.group(done2, None)
            done2 += 1
        pv_done = 0
        for J in range(NJ):
            a = J // NCK
            c = J % NCK
            s = s_next
            if J + 1 < NJ:
                s_next = adot(J + 1)
            if c == 0:
                mx = jnp.full((8, NQ), -jnp.inf, F32)
            for r in range(GPC):
                sg = s[r * G:(r + 1) * G]
                s_buf[a % 2, c * CK + r * G: c * CK + (r + 1) * G, :] = sg
                mx = jnp.maximum(mx, jnp.max(sg.reshape(G // 8, 8, NQ), axis=0))
                if c == NCK - 1 and r == GPC - 1:
                    s2.st['mfin'] = jnp.max(mx, axis=0, keepdims=True)
                gate = zgate(sg[0:8, 0:128])
                if r == 0 and J >= SCAN0 and (J - SCAN0) % SCANSTEP == 0 and (J - SCAN0) // SCANSTEP < SB // 8:
                    scan.step((J - SCAN0) // SCANSTEP, gate)
                target = min(ng, J * GPC + r + 1 + LEAD)
                while done2 < target and can2(done2, J, r):
                    s2.group(done2, gate)
                    done2 += 1
            last = NJ - 1 if J == NJ - 1 else NJ
            while pv_done < last and (pv_done + 1) * GPC <= done2 and pv_done <= J:
                s2.pv(pv_done)
                pv_done += 1
        y = _nt(scan.finish(), ccat[...])
        skip = (xb_blk.astype(F32) * coef[10, 0:1, :]).astype(BF16).astype(F32)
        y_stage[srows, :] = y + skip
        while pv_done < NJ:
            s2.pv(pv_done)
            pv_done += 1
        m_buf[...] = s2.st['mfin']
        vprev[...] = vc[(HPG - 1) * DH:HPG * DH, :]
        p_rows = pl.ds(pl.multiple_of((tp % NQB) * NQ, NQ), NQ)
        p_wo = wo[pl.ds(pl.multiple_of((tp // NQB) * 128, 128), 128), :]
        a_stage[p_rows, :] = a_stage[p_rows, :] + _tn(oT_prev[...], p_wo)
        oT_prev[0:(HPG - 1) * DH, :] = oT_cur[0:(HPG - 1) * DH, :]
        y_copy(t).start()

        @pl.when(t > (NG - 1) * NQB)
        def _():
            a_copy(tp % NQB).start()

        return carry

    lax.fori_loop(0, NB, attn, 0)

    wo_last = wo[(NG - 1) * 128:NG * 128, :]

    def last_softmax(n):
        cols = slice(n * 128, (n + 1) * 128)
        m = jnp.broadcast_to(m_buf[:, cols], (8, 128))
        l = jnp.zeros((8, 128), F32)
        o = jnp.zeros((DH, 128), F32)
        for c in range(NCK):
            p = jnp.exp2(s_buf[1, c * CK:(c + 1) * CK, cols].reshape(CK // 8, 8, 128) - m[None])
            l = l + jnp.sum(p, axis=0)
            o = o + _nn(vprev[:, c * CK:(c + 1) * CK], p.reshape(CK, 128).astype(BF16))
        oT_prev[(HPG - 1) * DH:HPG * DH, cols] = (o / jnp.sum(l, axis=0, keepdims=True)).astype(BF16)

    def last_proj(n):
        r0 = (NQB - 1) * NQ + n * 128
        a_stage[r0:r0 + 128, :] = a_stage[r0:r0 + 128, :] + _tn(oT_prev[:, n * 128:(n + 1) * 128], wo_last)
        return pltpu.make_async_copy(a_stage.at[pl.ds(r0, 128), :], out.at[pl.ds(r0, 128), pl.ds(0, D)], sem_a.at[NQB - 1 + n])

    tail = []
    last_softmax(0)
    for n in range(4):
        if n + 1 < 4:
            last_softmax(n + 1)
        cp = last_proj(n)
        cp.start()
        tail.append(cp)

    for t in range(NB):
        y_copy(t).wait()
    for qb_ in range(NQB - 1):
        a_copy(qb_).wait()
    for cp in tail:
        cp.wait()


@jax.jit
def pallas_concat_heads__softmax_full_mha__ssm_conv_s5__prompt_kernel(A_x, A_wqkv, A_wo, B_x, B_Lambda_re, B_Lambda_im, B_B_re, B_B_im, B_C_re, B_C_im, B_log_dt, B_Dskip):
    xa = A_x.reshape(S, D)
    xb = B_x.reshape(S, D)
    vm = pl.BlockSpec(memory_space=pltpu.VMEM)
    hbm = pl.BlockSpec(memory_space=pl.ANY)
    out = pl.pallas_call(
        _kernel,
        out_shape=jax.ShapeDtypeStruct((S, 2 * D), F32),
        in_specs=[hbm, hbm, hbm, hbm, vm, vm, hbm, hbm, hbm, hbm, vm, vm],
        out_specs=hbm,
        scratch_shapes=[
            pltpu.VMEM((S, D), BF16),
            pltpu.VMEM((D, 3 * D), BF16),
            pltpu.VMEM((D, D), BF16),
            pltpu.VMEM((S, D), BF16),
            pltpu.VMEM((2 * D, D), BF16),
            pltpu.VMEM((D, 2 * D), BF16),
            pltpu.VMEM((11, 8, D), F32),
            pltpu.VMEM((NG, S, 128), BF16),
            pltpu.VMEM((NRB, D, RB), BF16),
            pltpu.VMEM((NRB, D, RB), BF16),
            pltpu.VMEM((128, NQ), BF16),
            pltpu.VMEM((128, NQ), BF16),
            pltpu.VMEM((S, 128), BF16),
            pltpu.VMEM((128, S), BF16),
            pltpu.VMEM((DH, S), BF16),
            pltpu.VMEM((128, NQ), BF16),
            pltpu.VMEM((2, S, NQ), F32),
            pltpu.VMEM((1, NQ), F32),
            pltpu.VMEM((8, 128), I32),
            pltpu.VMEM((8, SB + 8, 128), F32),
            pltpu.VMEM((8, 8, 128), F32),
            pltpu.VMEM((S, D), F32),
            pltpu.VMEM((S, D), F32),
            pltpu.SemaphoreType.DMA((9,)),
            pltpu.SemaphoreType.DMA((NRB,)),
            pltpu.SemaphoreType.DMA((NB,)),
            pltpu.SemaphoreType.DMA((NQB + 3,)),
        ],
        compiler_params=pltpu.CompilerParams(vmem_limit_bytes=100 * 2 ** 20),
        name="fused_mha_s5",
    )(xa, A_wqkv, A_wo, xb, B_Lambda_re, B_Lambda_im, B_B_re, B_B_im, B_C_re, B_C_im, B_log_dt, B_Dskip)
    return out.reshape(1, S, 2 * D)
```

```python
import math

import jax
import jax.numpy as jnp
from jax import lax
from jax.experimental import pallas as pl
from jax.experimental.pallas import tpu as pltpu

S = 2048
D = 512
DH = 16
HPG = 8
NG = 4
NQ = 512
NQB = S // NQ
NB = NG * NQB
RB = 256
NRB = S // RB
SB = S // NB
CK = 128
NCK = S // CK
NKG = CK // 16
NJ = HPG * NCK
NT = NQ // 128
SH = 2
LA = 1
OFF = 2
USP = 2
PAT = '01'
ND = 2
OFF0 = 20
SCAN0 = 2
SCANSTEP = 1
FORCE_FALLBACK = 0
QSCALE = (DH ** -0.5) * math.log2(math.e)
L_SAFE = 2.0 ** -80

F32 = jnp.float32
BF16 = jnp.bfloat16
I32 = jnp.int32


def _nt(a, b):
    return lax.dot_general(a, b, (((1,), (1,)), ((), ())), preferred_element_type=F32)


def _tn(a, b):
    return lax.dot_general(a, b, (((0,), (0,)), ((), ())), preferred_element_type=F32)


def _nn(a, b):
    return jnp.dot(a, b, preferred_element_type=F32)


def _offl(J):
    return OFF > 0 and PAT[J % len(PAT)] == '1' and J >= max(USP, OFF0)


def _kernel(xa_h, wqkv_h, wo_h, xb_h, lre, lim, bre_h, bim_h, cre_h, cim_h, ldt, dsk, out,
            xa, wqkv, wo, xb, bcat, ccat, coef, k_all, qT_all, vT_all, oT_prev, oT_cur,
            kc, vc, wc, kf, qf, kn_scr, knb, sel, bad_scr, s_scr, zv, u_scr, h_scr, y_stage, a_stage,
            sem_w, sem_x, sem_y, sem_a):
    def x_copy(i):
        r = pl.ds(pl.multiple_of(i * RB, RB), RB)
        return pltpu.make_async_copy(xa_h.at[r, :], xa.at[r, :], sem_x.at[i])

    def wq_copy(n):
        c = pl.ds(n * D, D)
        return pltpu.make_async_copy(wqkv_h.at[:, c], wqkv.at[:, c], sem_w.at[n])

    w_copies = [
        pltpu.make_async_copy(bre_h, bcat.at[pl.ds(0, D), :], sem_w.at[3]),
        pltpu.make_async_copy(bim_h, bcat.at[pl.ds(D, D), :], sem_w.at[4]),
        pltpu.make_async_copy(xb_h, xb, sem_w.at[5]),
        pltpu.make_async_copy(cre_h, ccat.at[:, pl.ds(0, D)], sem_w.at[6]),
        pltpu.make_async_copy(cim_h, ccat.at[:, pl.ds(D, D)], sem_w.at[7]),
        pltpu.make_async_copy(wo_h, wo, sem_w.at[8]),
    ]
    x_copy(0).start()
    wq_copy(0).start()
    wq_copy(2).start()
    wq_copy(1).start()
    x_copy(1).start()

    zv[...] = jnp.zeros(zv.shape, I32)
    oT_prev[...] = jnp.zeros((128, NQ), BF16)
    a_stage[...] = jnp.zeros(a_stage.shape, F32)
    kn_scr[...] = jnp.zeros(kn_scr.shape, F32)
    bad_scr[...] = jnp.zeros(bad_scr.shape, F32)
    sel[...] = jnp.where(lax.broadcasted_iota(I32, (128, HPG * 128), 0) // DH
                         == lax.broadcasted_iota(I32, (128, HPG * 128), 1) // 128, 1.0, 0.0).astype(BF16)
    u_scr[:, 0:8, :] = jnp.zeros((8, 8, 128), F32)
    h_scr[...] = jnp.zeros(h_scr.shape, F32)

    l_re = lre[...].astype(F32).reshape(1, D)
    l_im = lim[...].astype(F32).reshape(1, D)
    dt = jnp.exp(ldt[...].astype(F32).reshape(1, D)).astype(BF16).astype(F32)
    e_re = dt * l_re
    e_im = dt * l_im

    def apow(k):
        mag = jnp.exp(k * e_re)
        return mag * jnp.cos(k * e_im), mag * jnp.sin(k * e_im)

    a1r, a1i = apow(1.0)
    for n, k in enumerate((1.0, 2.0, 4.0, 8.0)):
        r, i = apow(k)
        coef[2 * n] = jnp.broadcast_to(r, (8, D))
        coef[2 * n + 1] = jnp.broadcast_to(i, (8, D))
    nr = a1r - 1.0
    den = l_re * l_re + l_im * l_im
    coef[8] = jnp.broadcast_to(2.0 * (nr * l_re + a1i * l_im) / den, (8, D))
    coef[9] = jnp.broadcast_to(2.0 * (a1i * l_re - nr * l_im) / den, (8, D))
    coef[10] = jnp.broadcast_to(dsk[...].astype(F32).reshape(1, D), (8, D))

    def proj_q(i, xa_blk):
        qT_all[i] = (_nn(xa_blk, wqkv[:, 0:D]) * QSCALE).astype(BF16).T

    def proj_v(i, xa_blk):
        vT_all[i] = _nn(xa_blk, wqkv[:, 2 * D:3 * D]).astype(BF16).T

    def proj_k(rows, xa_blk):
        kb = _nn(xa_blk, wqkv[:, D:2 * D])
        kbb = kb.astype(BF16)
        for g in range(NG):
            k_all[g, rows, :] = kbb[:, g * 128:(g + 1) * 128]
        k2 = jnp.max((kb * kb).reshape(RB // 8, 8, D), axis=0)
        for g in range(NG):
            kn_scr[g] = jnp.maximum(kn_scr[g], k2[:, g * 128:(g + 1) * 128])

    x_copy(0).wait()
    wq_copy(0).wait()
    proj_q(0, xa[0:RB, :])
    wq_copy(2).wait()
    for i in range(2, NRB):
        x_copy(i).start()
    proj_v(0, xa[0:RB, :])
    wq_copy(1).wait()
    for cp in w_copies:
        cp.start()
    proj_k(pl.ds(0, RB), xa[0:RB, :])

    def proj(i, carry):
        x_copy(i).wait()
        rows = pl.ds(pl.multiple_of(i * RB, RB), RB)
        xa_blk = xa[rows, :]
        proj_q(i, xa_blk)
        proj_v(i, xa_blk)
        proj_k(rows, xa_blk)
        return carry

    lax.fori_loop(1, NRB, proj, 0)

    for g in range(NG):
        k2 = jnp.broadcast_to(jnp.max(kn_scr[g], axis=0, keepdims=True) * (1.0 + 2.0 ** -6), (8, 128))
        ks = _nn(k2.astype(BF16), sel[...])
        for j in range(HPG):
            knb[HPG * g + j] = ks[:, j * 128:(j + 1) * 128]

    for cp in w_copies:
        cp.wait()

    def wmat(j):
        parts = []
        if j > 0:
            parts.append(jnp.zeros((DH * j, NQ), BF16))
        parts.append(wc[j * DH:(j + 1) * DH, :])
        if j < HPG - 1:
            parts.append(jnp.zeros((DH * (HPG - 1 - j), NQ), BF16))
        return jnp.concatenate(parts, axis=0)

    def y_copy(t):
        r = pl.ds(pl.multiple_of(t * SB, SB), SB)
        return pltpu.make_async_copy(y_stage.at[r, :], out.at[r, pl.ds(D, D)], sem_y.at[t])

    def a_copy(qb_):
        r = pl.ds(pl.multiple_of(qb_ * NQ, NQ), NQ)
        return pltpu.make_async_copy(a_stage.at[r, :], out.at[r, pl.ds(0, D)], sem_a.at[qb_])

    rowid = lax.broadcasted_iota(I32, (8, 128), 0)

    class Scan:
        def __init__(self):
            self.prev = {}
            self.h = [(h_scr[c], h_scr[4 + c]) for c in range(4)]
            self.out = []

        def _fir(self, c, ur, ui, halo):
            lanes = slice(c * 128, (c + 1) * 128)
            wr, wi = ur, ui
            for n, k in enumerate((1, 2, 4)):
                rr = pltpu.roll(wr, k, 0)
                ri = pltpu.roll(wi, k, 0)
                if halo:
                    sr, si = rr, ri
                else:
                    pr, pi = self.prev[(c, n)]
                    sr = jnp.where(rowid < k, pr, rr)
                    si = jnp.where(rowid < k, pi, ri)
                self.prev[(c, n)] = (rr, ri)
                if halo and n == 2:
                    break
                ar = coef[2 * n, :, lanes]
                ai = coef[2 * n + 1, :, lanes]
                wr, wi = wr + ar * sr - ai * si, wi + ar * si + ai * sr
            return wr, wi

        def halo(self):
            for c in range(4):
                self._fir(c, u_scr[c, 0:8, :], u_scr[4 + c, 0:8, :], True)

        def step(self, tile, gate):
            rows = slice(8 + tile * 8, 16 + tile * 8)
            res = []
            for c in range(4):
                lanes = slice(c * 128, (c + 1) * 128)
                wr, wi = self._fir(c, u_scr[c, rows, :] + gate, u_scr[4 + c, rows, :] + gate, False)
                ar = coef[6, :, lanes]
                ai = coef[7, :, lanes]
                hr, hi = self.h[c]
                hr, hi = wr + ar * hr - ai * hi, wi + ar * hi + ai * hr
                self.h[c] = (hr, hi)
                fr = coef[8, :, lanes]
                fi = coef[9, :, lanes]
                res.append((fr * hr - fi * hi, -(fr * hi + fi * hr)))
            self.out.append(jnp.concatenate([r[0] for r in res] + [r[1] for r in res], axis=1))

        def finish(self):
            for c in range(4):
                h_scr[c] = self.h[c][0]
                h_scr[4 + c] = self.h[c][1]
            for c in range(8):
                u_scr[c, 0:8, :] = u_scr[c, SB:SB + 8, :]
            return jnp.concatenate(self.out, axis=0).astype(BF16)

    class Unit:
        def __init__(self, J):
            self.a, self.c, self.acc, self.d = J // NCK, J % NCK, None, 0

        def step(self, nd, gate):
            k16 = kf[self.c] + jnp.concatenate([gate, gate], axis=0)
            for d in range(self.d, self.d + nd):
                col = DH * self.a + d
                kb = jnp.broadcast_to(k16[:, col:col + 1], (16, NQ))
                q8 = jnp.concatenate([jnp.broadcast_to(qf[ct, col:col + 1, :], (8, 128)) for ct in range(NT)], axis=1)
                tt = kb * jnp.concatenate([q8, q8], axis=0)
                self.acc = tt if self.acc is None else self.acc + tt
            self.d += nd

    def attn(t, carry):
        g = t // NQB
        qbi = t % NQB
        tp = jnp.maximum(t - 1, 0)

        @pl.when(qbi == 0)
        def _():
            kc[...] = k_all[g]
            gr = pl.ds(pl.multiple_of(g * 128, 128), 128)
            for b in range(NRB):
                vc[:, b * RB:(b + 1) * RB] = vT_all[b, gr, :]
            if OFF > 0:
                for n in range(NCK):
                    kf[n] = k_all[g, n * CK:n * CK + 16, :].astype(F32)

        gr = pl.ds(pl.multiple_of(g * 128, 128), 128)
        wc[:, 0:RB] = qT_all[2 * qbi, gr, :]
        wc[:, RB:2 * RB] = qT_all[2 * qbi + 1, gr, :]
        for ct in range(NT):
            qf[ct] = wc[:, ct * 128:(ct + 1) * 128].astype(F32)

        srows = pl.ds(pl.multiple_of(t * SB, SB), SB)
        xb_blk = xb[srows, :]
        u = _nt(xb_blk, bcat[...])
        for c in range(8):
            u_scr[c, 8:8 + SB, :] = u[:, c * 128:(c + 1) * 128]
        scan = Scan()
        scan.halo()

        zi = zv[...]

        def zgate(x):
            return lax.bitcast_convert_type(lax.bitcast_convert_type(x, I32) & zi, F32)

        def order(J):
            return [x for x in range(NKG - 1, -1, -1) if not (x == 0 and _offl(J))]

        def dot_groups(J):
            a = J // NCK
            c = J % NCK
            st = [(cc, x) for cc in range(NCK) for x in order(a * NCK + cc)]
            pos = [i for i in range(len(st)) if i == 0 or st[i - 1][0] != st[i][0]]
            lo = 0 if c == 0 else pos[c] + SH
            hi = len(st) if c == NCK - 1 else pos[c + 1] + SH
            return st[lo:hi]

        def adot(J):
            lhs = jnp.concatenate([kc[c * CK + 16 * x:c * CK + 16 * (x + 1), :] for (c, x) in dot_groups(J)], axis=0)
            return _nn(lhs, wmat(J // NCK))

        def bound(j):
            q = jnp.concatenate([qf[ct, j * DH:(j + 1) * DH, :] for ct in range(NT)], axis=1)
            q2 = jnp.sum(q * q, axis=0, keepdims=True)
            kk = jnp.concatenate([knb[g * HPG + j][0:1]] * NT, axis=1)
            return jnp.broadcast_to(jnp.sqrt(q2 * kk), (8, NQ))

        def filler_y():
            y = _nt(scan.finish(), ccat[...])
            skip = (xb_blk.astype(F32) * coef[10, 0:1, :]).astype(BF16).astype(F32)
            y_stage[srows, :] = y + skip

        def filler_out():
            p_rows = pl.ds(pl.multiple_of((tp % NQB) * NQ, NQ), NQ)
            p_wo = wo[pl.ds(pl.multiple_of((tp // NQB) * 128, 128), 128), :]
            a_stage[p_rows, :] = a_stage[p_rows, :] + _tn(oT_prev[...], p_wo)

        pend = {J: adot(J) for J in range(LA)}
        units = {}
        ps = {}
        bad = jnp.zeros((1, NQ), F32)
        for J in range(NJ):
            a = J // NCK
            c = J % NCK
            if J + LA < NJ:
                pend[J + LA] = adot(J + LA)
            if J == NJ - 2:
                filler_y()
            if J == NJ - 1:
                filler_out()
            s = pend.pop(J)
            if c == 0:
                m = bound(a)
                l = jnp.zeros((8, NQ), F32)
                o = jnp.zeros((DH, NQ), F32)
            for i, (cc, x) in enumerate(dot_groups(J)):
                sg = s[16 * i:16 * (i + 1)]
                p = jnp.exp2(sg.reshape(2, 8, NQ) - m[None])
                l = l + p[0] + p[1]
                ps[(cc, x)] = p.reshape(16, NQ)
                if i % 2 == 0:
                    gate = zgate(sg[0:8, 0:128])
                    if i == 0 and J >= SCAN0 and (J - SCAN0) % SCANSTEP == 0 and (J - SCAN0) // SCANSTEP < SB // 8:
                        scan.step((J - SCAN0) // SCANSTEP, gate)
                    for Ju in range(J + 1, min(J + USP, NJ - 1) + 1):
                        if _offl(Ju):
                            if Ju not in units:
                                units[Ju] = Unit(Ju)
                            if units[Ju].d < DH:
                                units[Ju].step(min(ND, DH - units[Ju].d), gate)
                                break
            if _offl(J):
                un = units.pop(J)
                if un.d < DH:
                    un.step(DH - un.d, gate)
                p = jnp.exp2(un.acc.reshape(2, 8, NQ) - m[None])
                l = l + p[0] + p[1]
                ps[(c, 0)] = p.reshape(16, NQ)
            pb = jnp.concatenate([ps.pop((c, x)) for x in range(NKG)], axis=0).astype(BF16)
            o = o + _nn(vc[a * DH:(a + 1) * DH, c * CK:(c + 1) * CK], pb)
            if c == NCK - 1:
                lsum = jnp.sum(l, axis=0, keepdims=True)
                oT_cur[a * DH:(a + 1) * DH, :] = (o / lsum).astype(BF16)
                bad = jnp.maximum(bad, jnp.where(lsum >= L_SAFE, 0.0, 1.0))
        bad_scr[...] = jnp.maximum(bad_scr[...], bad)
        oT_prev[...] = oT_cur[...]
        y_copy(t).start()

        @pl.when(t > (NG - 1) * NQB)
        def _():
            a_copy(tp % NQB).start()

        return carry

    lax.fori_loop(0, NB, attn, 0)

    wo_last = wo[(NG - 1) * 128:NG * 128, :]
    tail = []
    for n in range(4):
        r0 = (NQB - 1) * NQ + n * 128
        a_stage[r0:r0 + 128, :] = a_stage[r0:r0 + 128, :] + _tn(oT_prev[:, n * 128:(n + 1) * 128], wo_last)
        cp = pltpu.make_async_copy(a_stage.at[pl.ds(r0, 128), :], out.at[pl.ds(r0, 128), pl.ds(0, D)], sem_a.at[NQB - 1 + n])
        cp.start()
        tail.append(cp)

    for t in range(NB):
        y_copy(t).wait()
    for qb_ in range(NQB - 1):
        a_copy(qb_).wait()
    for cp in tail:
        cp.wait()

    unsafe = jnp.max(bad_scr[...]) > (-1.0 if FORCE_FALLBACK else 0.5)

    @pl.when(unsafe)
    def _():
        headid = lax.broadcasted_iota(I32, (128, NQ), 0) // DH

        def fb_body(t, carry):
            g = t // NQB
            qbi = t % NQB
            gr = pl.ds(pl.multiple_of(g * 128, 128), 128)
            wc[:, 0:RB] = qT_all[2 * qbi, gr, :]
            wc[:, RB:2 * RB] = qT_all[2 * qbi + 1, gr, :]

            def fb_head(j, carry2):
                wj = jnp.where(headid == j, wc[...].astype(F32), 0.0).astype(BF16)

                def pass1(b, m):
                    rows = pl.ds(pl.multiple_of(b * RB, RB), RB)
                    s = _nn(k_all[g, rows, :], wj)
                    s_scr[rows, :] = s
                    return jnp.maximum(m, jnp.max(s, axis=0, keepdims=True))

                m = lax.fori_loop(0, NRB, pass1, jnp.full((1, NQ), -jnp.inf, F32))

                def pass2(b, lo):
                    rows = pl.ds(pl.multiple_of(b * RB, RB), RB)
                    p = jnp.exp2(s_scr[rows, :] - m)
                    hr = pl.ds(pl.multiple_of(g * 128 + j * DH, DH), DH)
                    return (lo[0] + jnp.sum(p, axis=0, keepdims=True),
                            lo[1] + _nn(vT_all[b, hr, :], p.astype(BF16)))

                l, o = lax.fori_loop(0, NRB, pass2, (jnp.zeros((1, NQ), F32), jnp.zeros((DH, NQ), F32)))
                oT_cur[pl.ds(pl.multiple_of(j * DH, DH), DH), :] = (o / l).astype(BF16)
                return carry2

            lax.fori_loop(0, HPG, fb_head, 0)
            rows = pl.ds(pl.multiple_of(qbi * NQ, NQ), NQ)
            part = _tn(oT_cur[...], wo[gr, :])
            a_stage[rows, :] = jnp.where(g == 0, 0.0, a_stage[rows, :]) + part
            return carry

        lax.fori_loop(0, NB, fb_body, 0)
        cps = [a_copy(qb_) for qb_ in range(NQB)]
        for cp in cps:
            cp.start()
        for cp in cps:
            cp.wait()


@jax.jit
def pallas_concat_heads__softmax_full_mha__ssm_conv_s5__prompt_kernel(A_x, A_wqkv, A_wo, B_x, B_Lambda_re, B_Lambda_im, B_B_re, B_B_im, B_C_re, B_C_im, B_log_dt, B_Dskip):
    xa = A_x.reshape(S, D)
    xb = B_x.reshape(S, D)
    vm = pl.BlockSpec(memory_space=pltpu.VMEM)
    hbm = pl.BlockSpec(memory_space=pl.ANY)
    out = pl.pallas_call(
        _kernel,
        out_shape=jax.ShapeDtypeStruct((S, 2 * D), F32),
        in_specs=[hbm, hbm, hbm, hbm, vm, vm, hbm, hbm, hbm, hbm, vm, vm],
        out_specs=hbm,
        scratch_shapes=[
            pltpu.VMEM((S, D), BF16),
            pltpu.VMEM((D, 3 * D), BF16),
            pltpu.VMEM((D, D), BF16),
            pltpu.VMEM((S, D), BF16),
            pltpu.VMEM((2 * D, D), BF16),
            pltpu.VMEM((D, 2 * D), BF16),
            pltpu.VMEM((11, 8, D), F32),
            pltpu.VMEM((NG, S, 128), BF16),
            pltpu.VMEM((NRB, D, RB), BF16),
            pltpu.VMEM((NRB, D, RB), BF16),
            pltpu.VMEM((128, NQ), BF16),
            pltpu.VMEM((128, NQ), BF16),
            pltpu.VMEM((S, 128), BF16),
            pltpu.VMEM((128, S), BF16),
            pltpu.VMEM((128, NQ), BF16),
            pltpu.VMEM((NCK, 16, 128), F32),
            pltpu.VMEM((NT, 128, 128), F32),
            pltpu.VMEM((NG, 8, 128), F32),
            pltpu.VMEM((NG * HPG, 8, 128), F32),
            pltpu.VMEM((128, HPG * 128), BF16),
            pltpu.VMEM((1, NQ), F32),
            pltpu.VMEM((S, NQ), F32),
            pltpu.VMEM((8, 128), I32),
            pltpu.VMEM((8, SB + 8, 128), F32),
            pltpu.VMEM((8, 8, 128), F32),
            pltpu.VMEM((S, D), F32),
            pltpu.VMEM((S, D), F32),
            pltpu.SemaphoreType.DMA((9,)),
            pltpu.SemaphoreType.DMA((NRB,)),
            pltpu.SemaphoreType.DMA((NB,)),
            pltpu.SemaphoreType.DMA((NQB + 3,)),
        ],
        compiler_params=pltpu.CompilerParams(vmem_limit_bytes=100 * 2 ** 20),
        name="fused_mha_s5",
    )(xa, A_wqkv, A_wo, xb, B_Lambda_re, B_Lambda_im, B_B_re, B_B_im, B_C_re, B_C_im, B_log_dt, B_Dskip)
    return out.reshape(1, S, 2 * D)
```

```python
import math

import jax
import jax.numpy as jnp
from jax import lax
from jax.experimental import pallas as pl
from jax.experimental.pallas import tpu as pltpu

S = 2048
D = 512
DH = 16
HPG = 8
NG = 4
NQ = 512
NQB = S // NQ
NB = NG * NQB
RB = 256
NRB = S // RB
SB = S // NB
CK = 128
NCK = S // CK
NKG = CK // 16
NJ = HPG * NCK
NT = NQ // 128
SH = 2
LA = 1
OFF = 2
USP = 2
PAT = '01'
ND = 2
MNEXT = 8
HOLD = 1
EARLY = 1
DLJ = -1
OFF0 = 2
SCAN0 = 8
SCANSTEP = 7
FORCE_FALLBACK = 0
QSCALE = (DH ** -0.5) * math.log2(math.e)
L_SAFE = 2.0 ** -80

F32 = jnp.float32
BF16 = jnp.bfloat16
I32 = jnp.int32


def _nt(a, b):
    return lax.dot_general(a, b, (((1,), (1,)), ((), ())), preferred_element_type=F32)


def _tn(a, b):
    return lax.dot_general(a, b, (((0,), (0,)), ((), ())), preferred_element_type=F32)


def _nn(a, b):
    return jnp.dot(a, b, preferred_element_type=F32)


def _offl(J):
    return OFF > 0 and PAT[J % len(PAT)] == '1' and J >= max(USP, OFF0)


def _kernel(xa_h, wqkv_h, wo_h, xb_h, lre, lim, bre_h, bim_h, cre_h, cim_h, ldt, dsk, out,
            xa, wqkv, wo, xb, bcat, ccat, coef, k_all, qT_all, vT_all, oT_prev, oT_cur,
            kc, vc, wc, kf, qf, kn_scr, knb, sel, bad_scr, s_scr, zv, u_scr, h_scr, y_stage, a_stage,
            sem_w, sem_x, sem_y, sem_a):
    def x_copy(i):
        r = pl.ds(pl.multiple_of(i * RB, RB), RB)
        return pltpu.make_async_copy(xa_h.at[r, :], xa.at[r, :], sem_x.at[i])

    def wq_copy(n):
        c = pl.ds(n * D, D)
        return pltpu.make_async_copy(wqkv_h.at[:, c], wqkv.at[:, c], sem_w.at[n])

    w_copies = [
        pltpu.make_async_copy(bre_h, bcat.at[pl.ds(0, D), :], sem_w.at[3]),
        pltpu.make_async_copy(bim_h, bcat.at[pl.ds(D, D), :], sem_w.at[4]),
        pltpu.make_async_copy(xb_h, xb, sem_w.at[5]),
        pltpu.make_async_copy(cre_h, ccat.at[:, pl.ds(0, D)], sem_w.at[6]),
        pltpu.make_async_copy(cim_h, ccat.at[:, pl.ds(D, D)], sem_w.at[7]),
        pltpu.make_async_copy(wo_h, wo, sem_w.at[8]),
    ]
    x_copy(0).start()
    wq_copy(0).start()
    wq_copy(2).start()
    wq_copy(1).start()
    x_copy(1).start()

    zv[...] = jnp.zeros(zv.shape, I32)
    oT_prev[...] = jnp.zeros((128, NQ), BF16)
    a_stage[...] = jnp.zeros(a_stage.shape, F32)
    kn_scr[...] = jnp.zeros(kn_scr.shape, F32)
    bad_scr[...] = jnp.zeros(bad_scr.shape, F32)
    sel[...] = jnp.where(lax.broadcasted_iota(I32, (128, HPG * 128), 0) // DH
                         == lax.broadcasted_iota(I32, (128, HPG * 128), 1) // 128, 1.0, 0.0).astype(BF16)
    u_scr[:, 0:8, :] = jnp.zeros((8, 8, 128), F32)
    h_scr[...] = jnp.zeros(h_scr.shape, F32)

    l_re = lre[...].astype(F32).reshape(1, D)
    l_im = lim[...].astype(F32).reshape(1, D)
    dt = jnp.exp(ldt[...].astype(F32).reshape(1, D)).astype(BF16).astype(F32)
    e_re = dt * l_re
    e_im = dt * l_im

    def apow(k):
        mag = jnp.exp(k * e_re)
        return mag * jnp.cos(k * e_im), mag * jnp.sin(k * e_im)

    a1r, a1i = apow(1.0)
    for n, k in enumerate((1.0, 2.0, 4.0, 8.0)):
        r, i = apow(k)
        coef[2 * n] = jnp.broadcast_to(r, (8, D))
        coef[2 * n + 1] = jnp.broadcast_to(i, (8, D))
    nr = a1r - 1.0
    den = l_re * l_re + l_im * l_im
    coef[8] = jnp.broadcast_to(2.0 * (nr * l_re + a1i * l_im) / den, (8, D))
    coef[9] = jnp.broadcast_to(2.0 * (a1i * l_re - nr * l_im) / den, (8, D))
    coef[10] = jnp.broadcast_to(dsk[...].astype(F32).reshape(1, D), (8, D))

    def proj_q(i, xa_blk):
        qT_all[i] = (_nn(xa_blk, wqkv[:, 0:D]) * QSCALE).astype(BF16).T

    def proj_v(i, xa_blk):
        vT_all[i] = _nn(xa_blk, wqkv[:, 2 * D:3 * D]).astype(BF16).T

    def proj_k(rows, xa_blk):
        kb = _nn(xa_blk, wqkv[:, D:2 * D])
        kbb = kb.astype(BF16)
        for g in range(NG):
            k_all[g, rows, :] = kbb[:, g * 128:(g + 1) * 128]
        k2 = jnp.max((kb * kb).reshape(RB // 8, 8, D), axis=0)
        for g in range(NG):
            kn_scr[g] = jnp.maximum(kn_scr[g], k2[:, g * 128:(g + 1) * 128])

    x_copy(0).wait()
    wq_copy(0).wait()
    proj_q(0, xa[0:RB, :])
    wq_copy(2).wait()
    for i in range(2, NRB):
        x_copy(i).start()
    proj_v(0, xa[0:RB, :])
    wq_copy(1).wait()
    for cp in w_copies:
        cp.start()
    proj_k(pl.ds(0, RB), xa[0:RB, :])

    def proj(i, carry):
        x_copy(i).wait()
        rows = pl.ds(pl.multiple_of(i * RB, RB), RB)
        xa_blk = xa[rows, :]
        proj_q(i, xa_blk)
        proj_v(i, xa_blk)
        proj_k(rows, xa_blk)
        return carry

    lax.fori_loop(1, NRB, proj, 0)

    for g in range(NG):
        k2 = jnp.broadcast_to(jnp.max(kn_scr[g], axis=0, keepdims=True) * (1.0 + 2.0 ** -6), (8, 128))
        ks = _nn(k2.astype(BF16), sel[...])
        for j in range(HPG):
            knb[HPG * g + j] = ks[:, j * 128:(j + 1) * 128]

    for cp in w_copies:
        cp.wait()

    def wmat(j):
        parts = []
        if j > 0:
            parts.append(jnp.zeros((DH * j, NQ), BF16))
        parts.append(wc[j * DH:(j + 1) * DH, :])
        if j < HPG - 1:
            parts.append(jnp.zeros((DH * (HPG - 1 - j), NQ), BF16))
        return jnp.concatenate(parts, axis=0)

    def y_copy(t):
        r = pl.ds(pl.multiple_of(t * SB, SB), SB)
        return pltpu.make_async_copy(y_stage.at[r, :], out.at[r, pl.ds(D, D)], sem_y.at[t])

    def a_copy(qb_):
        r = pl.ds(pl.multiple_of(qb_ * NQ, NQ), NQ)
        return pltpu.make_async_copy(a_stage.at[r, :], out.at[r, pl.ds(0, D)], sem_a.at[qb_])

    rowid = lax.broadcasted_iota(I32, (8, 128), 0)

    class Scan:
        def __init__(self):
            self.prev = {}
            self.h = [(h_scr[c], h_scr[4 + c]) for c in range(4)]
            self.out = []

        def _fir(self, c, ur, ui, halo):
            lanes = slice(c * 128, (c + 1) * 128)
            wr, wi = ur, ui
            for n, k in enumerate((1, 2, 4)):
                rr = pltpu.roll(wr, k, 0)
                ri = pltpu.roll(wi, k, 0)
                if halo:
                    sr, si = rr, ri
                else:
                    pr, pi = self.prev[(c, n)]
                    sr = jnp.where(rowid < k, pr, rr)
                    si = jnp.where(rowid < k, pi, ri)
                self.prev[(c, n)] = (rr, ri)
                if halo and n == 2:
                    break
                ar = coef[2 * n, :, lanes]
                ai = coef[2 * n + 1, :, lanes]
                wr, wi = wr + ar * sr - ai * si, wi + ar * si + ai * sr
            return wr, wi

        def halo(self):
            for c in range(4):
                self._fir(c, u_scr[c, 0:8, :], u_scr[4 + c, 0:8, :], True)

        def step(self, tile, gate):
            rows = slice(8 + tile * 8, 16 + tile * 8)
            res = []
            for c in range(4):
                lanes = slice(c * 128, (c + 1) * 128)
                wr, wi = self._fir(c, u_scr[c, rows, :] + gate, u_scr[4 + c, rows, :] + gate, False)
                ar = coef[6, :, lanes]
                ai = coef[7, :, lanes]
                hr, hi = self.h[c]
                hr, hi = wr + ar * hr - ai * hi, wi + ar * hi + ai * hr
                self.h[c] = (hr, hi)
                fr = coef[8, :, lanes]
                fi = coef[9, :, lanes]
                res.append((fr * hr - fi * hi, -(fr * hi + fi * hr)))
            self.out.append(jnp.concatenate([r[0] for r in res] + [r[1] for r in res], axis=1))

        def finish(self):
            for c in range(4):
                h_scr[c] = self.h[c][0]
                h_scr[4 + c] = self.h[c][1]
            for c in range(8):
                u_scr[c, 0:8, :] = u_scr[c, SB:SB + 8, :]
            return jnp.concatenate(self.out, axis=0).astype(BF16)

    def ssm_scan_lane(c):
        lanes = slice(c * 128, (c + 1) * 128)
        prev = {}

        def fir(ur, ui, halo):
            wr, wi = ur, ui
            for n, k in enumerate((1, 2, 4)):
                rr = pltpu.roll(wr, k, 0)
                ri = pltpu.roll(wi, k, 0)
                if halo:
                    sr, si = rr, ri
                else:
                    pr, pi = prev[n]
                    sr = jnp.where(rowid < k, pr, rr)
                    si = jnp.where(rowid < k, pi, ri)
                prev[n] = (rr, ri)
                if halo and n == 2:
                    break
                ar = coef[2 * n, :, lanes]
                ai = coef[2 * n + 1, :, lanes]
                wr, wi = wr + ar * sr - ai * si, wi + ar * si + ai * sr
            return wr, wi

        fir(u_scr[c, 0:8, :], u_scr[4 + c, 0:8, :], True)
        hr, hi = h_scr[c], h_scr[4 + c]
        outr, outi = [], []
        for tile in range(SB // 8):
            rows = slice(8 + tile * 8, 16 + tile * 8)
            wr, wi = fir(u_scr[c, rows, :], u_scr[4 + c, rows, :], False)
            ar = coef[6, :, lanes]
            ai = coef[7, :, lanes]
            hr, hi = wr + ar * hr - ai * hi, wi + ar * hi + ai * hr
            fr = coef[8, :, lanes]
            fi = coef[9, :, lanes]
            outr.append(fr * hr - fi * hi)
            outi.append(-(fr * hi + fi * hr))
        h_scr[c] = hr
        h_scr[4 + c] = hi
        u_scr[c, 0:8, :] = u_scr[c, SB:SB + 8, :]
        u_scr[4 + c, 0:8, :] = u_scr[4 + c, SB:SB + 8, :]
        return (jnp.concatenate(outr, axis=0).astype(BF16), jnp.concatenate(outi, axis=0).astype(BF16),
                [hr, hi, outr[-1], outi[-1]])

    class Unit:
        def __init__(self, J):
            self.a, self.c, self.acc, self.d = J // NCK, J % NCK, None, 0

        def step(self, nd, gate):
            k16 = kf[self.c] + jnp.concatenate([gate, gate], axis=0)
            for d in range(self.d, self.d + nd):
                col = DH * self.a + d
                kb = jnp.broadcast_to(k16[:, col:col + 1], (16, NQ))
                q8 = jnp.concatenate([jnp.broadcast_to(qf[ct, col:col + 1, :], (8, 128)) for ct in range(NT)], axis=1)
                tt = kb * jnp.concatenate([q8, q8], axis=0)
                self.acc = tt if self.acc is None else self.acc + tt
            self.d += nd

    def attn(t, carry):
        g = t // NQB
        qbi = t % NQB
        tp = jnp.maximum(t - 1, 0)

        @pl.when(qbi == 0)
        def _():
            kc[...] = k_all[g]
            gr = pl.ds(pl.multiple_of(g * 128, 128), 128)
            for b in range(NRB):
                vc[:, b * RB:(b + 1) * RB] = vT_all[b, gr, :]
            if OFF > 0:
                for n in range(NCK):
                    kf[n] = k_all[g, n * CK:n * CK + 16, :].astype(F32)

        @pl.when(t == NB - 1)
        def _():
            rows = pl.ds((NQB - 2) * NQ, NQ)
            a_stage[rows, :] = a_stage[rows, :] + _tn(oT_prev[...], wo[(NG - 1) * 128:NG * 128, :])
            a_copy(NQB - 2).start()

        gr = pl.ds(pl.multiple_of(g * 128, 128), 128)
        wc[:, 0:RB] = qT_all[2 * qbi, gr, :]
        wc[:, RB:2 * RB] = qT_all[2 * qbi + 1, gr, :]
        for ct in range(NT):
            qf[ct] = wc[:, ct * 128:(ct + 1) * 128].astype(F32)

        srows = pl.ds(pl.multiple_of(t * SB, SB), SB)
        xb_blk = xb[srows, :]
        if EARLY:
            hcols = {}
            hfin = []
            for c in range(4):
                bc = jnp.concatenate([bcat[c * 128:(c + 1) * 128, :], bcat[D + c * 128:D + (c + 1) * 128, :]], axis=0)
                uc = _nt(xb_blk, bc)
                u_scr[c, 8:8 + SB, :] = uc[:, 0:128]
                u_scr[4 + c, 8:8 + SB, :] = uc[:, 128:256]
            for c in range(4):
                hcols[c], hcols[4 + c], fin = ssm_scan_lane(c)
                hfin += fin
        else:
            u = _nt(xb_blk, bcat[...])
            for c in range(8):
                u_scr[c, 8:8 + SB, :] = u[:, c * 128:(c + 1) * 128]
            scan = Scan()
            scan.halo()

        zi = zv[...]

        def zgate(*xs):
            b = lax.bitcast_convert_type(xs[0], I32)
            for x in xs[1:]:
                b = b | lax.bitcast_convert_type(x, I32)
            return lax.bitcast_convert_type(b & zi, F32)

        def order(J):
            return [x for x in range(NKG - 1, -1, -1) if not (x == 0 and _offl(J))]

        def dot_groups(J):
            a = J // NCK
            c = J % NCK
            st = [(cc, x) for cc in range(NCK) for x in order(a * NCK + cc)]
            pos = [i for i in range(len(st)) if i == 0 or st[i - 1][0] != st[i][0]]
            lo = 0 if c == 0 else pos[c] + SH
            hi = len(st) if c == NCK - 1 else pos[c + 1] + SH
            return st[lo:hi]

        def adot(J):
            lhs = jnp.concatenate([kc[c * CK + 16 * x:c * CK + 16 * (x + 1), :] for (c, x) in dot_groups(J)], axis=0)
            return _nn(lhs, wmat(J // NCK))

        def bound(j):
            q = jnp.concatenate([qf[ct, j * DH:(j + 1) * DH, :] for ct in range(NT)], axis=1)
            q2 = jnp.sum(q * q, axis=0, keepdims=True)
            kk = jnp.concatenate([knb[g * HPG + j][0:1]] * NT, axis=1)
            return jnp.broadcast_to(jnp.sqrt(q2 * kk), (8, NQ))

        def filler_y():
            hcat = jnp.concatenate([hcols[c] for c in range(8)], axis=1) if EARLY else scan.finish()
            y = _nt(hcat, ccat[...])
            skip = (xb_blk.astype(F32) * coef[10, 0:1, :]).astype(BF16).astype(F32)
            y_stage[srows, :] = y + skip

        def filler_out():
            last = t == NB - 1
            p_rows = pl.ds(pl.multiple_of(jnp.where(last, NQB - 1, tp % NQB) * NQ, NQ), NQ)
            p_wo = wo[pl.ds(pl.multiple_of((tp // NQB) * 128, 128), 128), :]
            part = _tn(oT_prev[...], p_wo)
            a_stage[p_rows, :] = a_stage[p_rows, :] + jnp.where(last, 0.0, part)

        st = {}

        def pv(J):
            a = J // NCK
            c = J % NCK
            pb = jnp.concatenate([ps.pop((c, x)) for x in range(NKG)], axis=0).astype(BF16)
            o = _nn(vc[a * DH:(a + 1) * DH, c * CK:(c + 1) * CK], pb)
            st[('o', a)] = o if c == 0 else st[('o', a)] + o
            if c == NCK - 1:
                lsum = jnp.sum(st.pop(('l', a)), axis=0, keepdims=True)
                oT_cur[a * DH:(a + 1) * DH, :] = (st.pop(('o', a)) / lsum).astype(BF16)
                st['bad'] = jnp.maximum(st['bad'], jnp.where(lsum >= L_SAFE, 0.0, 1.0))

        pend = {J: adot(J) for J in range(LA)}
        units = {}
        ps = {}
        st['bad'] = jnp.zeros((1, NQ), F32)
        for J in range(NJ):
            a = J // NCK
            c = J % NCK
            if J + LA < NJ:
                pend[J + LA] = adot(J + LA)
            if HOLD and c == NCK - 1:
                if J == NJ - 1:
                    filler_y()
                pv(J - 1)
            if J == NJ - 2 and not HOLD:
                filler_y()
            if J == NJ - 1:
                filler_out()
            s = pend.pop(J)
            if EARLY and J == DLJ:
                m = m + jnp.concatenate([zgate(*hfin)] * NT, axis=1)
            if c == MNEXT and a + 1 < HPG:
                m_next = bound(a + 1)
                m = m + jnp.concatenate([zgate(m_next[:, ct * 128:(ct + 1) * 128]) for ct in range(NT)], axis=1)
            if c == 0:
                m = bound(a) if (a == 0 or MNEXT < 0) else m_next
                l = jnp.zeros((8, NQ), F32)
            for i, (cc, x) in enumerate(dot_groups(J)):
                sg = s[16 * i:16 * (i + 1)]
                p = jnp.exp2(sg.reshape(2, 8, NQ) - m[None])
                l = l + p[0] + p[1]
                ps[(cc, x)] = p.reshape(16, NQ)
                if i % 2 == 0:
                    gate = zgate(sg[0:8, 0:128])
                    if not EARLY and i == 0 and J >= SCAN0 and (J - SCAN0) % SCANSTEP == 0 and (J - SCAN0) // SCANSTEP < SB // 8:
                        scan.step((J - SCAN0) // SCANSTEP, gate)
                    for Ju in range(J + 1, min(J + USP, NJ - 1) + 1):
                        if _offl(Ju):
                            if Ju not in units:
                                units[Ju] = Unit(Ju)
                            if units[Ju].d < DH:
                                units[Ju].step(min(ND, DH - units[Ju].d), gate)
                                break
            if _offl(J):
                un = units.pop(J)
                if un.d < DH:
                    un.step(DH - un.d, gate)
                p = jnp.exp2(un.acc.reshape(2, 8, NQ) - m[None])
                l = l + p[0] + p[1]
                ps[(c, 0)] = p.reshape(16, NQ)
            st[('l', a)] = l
            if c != NCK - 2 or not HOLD:
                pv(J)
        bad_scr[...] = jnp.maximum(bad_scr[...], st['bad'])
        oT_prev[...] = oT_cur[...]
        y_copy(t).start()

        @pl.when((t > (NG - 1) * NQB) & (t < NB - 1))
        def _():
            a_copy(tp % NQB).start()

        return carry

    lax.fori_loop(0, NB, attn, 0)

    wo_last = wo[(NG - 1) * 128:NG * 128, :]
    tail = []
    for n in range(4):
        r0 = (NQB - 1) * NQ + n * 128
        a_stage[r0:r0 + 128, :] = a_stage[r0:r0 + 128, :] + _tn(oT_prev[:, n * 128:(n + 1) * 128], wo_last)
        cp = pltpu.make_async_copy(a_stage.at[pl.ds(r0, 128), :], out.at[pl.ds(r0, 128), pl.ds(0, D)], sem_a.at[NQB - 1 + n])
        cp.start()
        tail.append(cp)

    for t in range(NB):
        y_copy(t).wait()
    for qb_ in range(NQB - 1):
        a_copy(qb_).wait()
    for cp in tail:
        cp.wait()

    unsafe = jnp.max(bad_scr[...]) > (-1.0 if FORCE_FALLBACK else 0.5)

    @pl.when(unsafe)
    def _():
        headid = lax.broadcasted_iota(I32, (128, NQ), 0) // DH

        def fb_body(t, carry):
            g = t // NQB
            qbi = t % NQB
            gr = pl.ds(pl.multiple_of(g * 128, 128), 128)
            wc[:, 0:RB] = qT_all[2 * qbi, gr, :]
            wc[:, RB:2 * RB] = qT_all[2 * qbi + 1, gr, :]

            def fb_head(j, carry2):
                wj = jnp.where(headid == j, wc[...].astype(F32), 0.0).astype(BF16)

                def pass1(b, m):
                    rows = pl.ds(pl.multiple_of(b * RB, RB), RB)
                    s = _nn(k_all[g, rows, :], wj)
                    s_scr[rows, :] = s
                    return jnp.maximum(m, jnp.max(s, axis=0, keepdims=True))

                m = lax.fori_loop(0, NRB, pass1, jnp.full((1, NQ), -jnp.inf, F32))

                def pass2(b, lo):
                    rows = pl.ds(pl.multiple_of(b * RB, RB), RB)
                    p = jnp.exp2(s_scr[rows, :] - m)
                    hr = pl.ds(pl.multiple_of(g * 128 + j * DH, DH), DH)
                    return (lo[0] + jnp.sum(p, axis=0, keepdims=True),
                            lo[1] + _nn(vT_all[b, hr, :], p.astype(BF16)))

                l, o = lax.fori_loop(0, NRB, pass2, (jnp.zeros((1, NQ), F32), jnp.zeros((DH, NQ), F32)))
                oT_cur[pl.ds(pl.multiple_of(j * DH, DH), DH), :] = (o / l).astype(BF16)
                return carry2

            lax.fori_loop(0, HPG, fb_head, 0)
            rows = pl.ds(pl.multiple_of(qbi * NQ, NQ), NQ)
            part = _tn(oT_cur[...], wo[gr, :])
            a_stage[rows, :] = jnp.where(g == 0, 0.0, a_stage[rows, :]) + part
            return carry

        lax.fori_loop(0, NB, fb_body, 0)
        cps = [a_copy(qb_) for qb_ in range(NQB)]
        for cp in cps:
            cp.start()
        for cp in cps:
            cp.wait()


@jax.jit
def pallas_concat_heads__softmax_full_mha__ssm_conv_s5__prompt_kernel(A_x, A_wqkv, A_wo, B_x, B_Lambda_re, B_Lambda_im, B_B_re, B_B_im, B_C_re, B_C_im, B_log_dt, B_Dskip):
    xa = A_x.reshape(S, D)
    xb = B_x.reshape(S, D)
    vm = pl.BlockSpec(memory_space=pltpu.VMEM)
    hbm = pl.BlockSpec(memory_space=pl.ANY)
    out = pl.pallas_call(
        _kernel,
        out_shape=jax.ShapeDtypeStruct((S, 2 * D), F32),
        in_specs=[hbm, hbm, hbm, hbm, vm, vm, hbm, hbm, hbm, hbm, vm, vm],
        out_specs=hbm,
        scratch_shapes=[
            pltpu.VMEM((S, D), BF16),
            pltpu.VMEM((D, 3 * D), BF16),
            pltpu.VMEM((D, D), BF16),
            pltpu.VMEM((S, D), BF16),
            pltpu.VMEM((2 * D, D), BF16),
            pltpu.VMEM((D, 2 * D), BF16),
            pltpu.VMEM((11, 8, D), F32),
            pltpu.VMEM((NG, S, 128), BF16),
            pltpu.VMEM((NRB, D, RB), BF16),
            pltpu.VMEM((NRB, D, RB), BF16),
            pltpu.VMEM((128, NQ), BF16),
            pltpu.VMEM((128, NQ), BF16),
            pltpu.VMEM((S, 128), BF16),
            pltpu.VMEM((128, S), BF16),
            pltpu.VMEM((128, NQ), BF16),
            pltpu.VMEM((NCK, 16, 128), F32),
            pltpu.VMEM((NT, 128, 128), F32),
            pltpu.VMEM((NG, 8, 128), F32),
            pltpu.VMEM((NG * HPG, 8, 128), F32),
            pltpu.VMEM((128, HPG * 128), BF16),
            pltpu.VMEM((1, NQ), F32),
            pltpu.VMEM((S, NQ), F32),
            pltpu.VMEM((8, 128), I32),
            pltpu.VMEM((8, SB + 8, 128), F32),
            pltpu.VMEM((8, 8, 128), F32),
            pltpu.VMEM((S, D), F32),
            pltpu.VMEM((S, D), F32),
            pltpu.SemaphoreType.DMA((9,)),
            pltpu.SemaphoreType.DMA((NRB,)),
            pltpu.SemaphoreType.DMA((NB,)),
            pltpu.SemaphoreType.DMA((NQB + 3,)),
        ],
        compiler_params=pltpu.CompilerParams(vmem_limit_bytes=100 * 2 ** 20),
        name="fused_mha_s5",
    )(xa, A_wqkv, A_wo, xb, B_Lambda_re, B_Lambda_im, B_B_re, B_B_im, B_C_re, B_C_im, B_log_dt, B_Dskip)
    return out.reshape(1, S, 2 * D)
```

```python
import math

import jax
import jax.numpy as jnp
from jax import lax
from jax.experimental import pallas as pl
from jax.experimental.pallas import tpu as pltpu

S = 2048
D = 512
DH = 16
HPG = 8
NG = 4
NQ = 512
NQB = S // NQ
NB = NG * NQB
RB = 256
NRB = S // RB
SB = S // NB
CK = 128
NCK = S // CK
NKG = CK // 16
NJ = HPG * NCK
NT = NQ // 128
SHIFT = 2
VPU_SPAN = 2
VPU_DIMS = 2
BOUND_AT = 8
QSCALE = (DH ** -0.5) * math.log2(math.e)
L_SAFE = 2.0 ** -60

F32 = jnp.float32
BF16 = jnp.bfloat16
I32 = jnp.int32


def _nt(a, b):
    return lax.dot_general(a, b, (((1,), (1,)), ((), ())), preferred_element_type=F32)


def _tn(a, b):
    return lax.dot_general(a, b, (((0,), (0,)), ((), ())), preferred_element_type=F32)


def _nn(a, b):
    return jnp.dot(a, b, preferred_element_type=F32)


def _on_vpu(J):
    return J % 2 == 1 and J >= VPU_SPAN


def _kernel(xa_h, wqkv_h, wo_h, xb_h, lre, lim, bre_h, bim_h, cre_h, cim_h, ldt, dsk, out,
            xa, wqkv, wo, xb, bcat, ccat, coef, k_all, qT_all, vT_all, oT_prev, oT_cur,
            kc, vc, wc, kf, qf, kn_scr, knb, sel, bad_scr, s_scr, zv, u_scr, h_scr, y_stage, a_stage,
            sem_w, sem_x, sem_y, sem_a):
    def x_copy(i):
        r = pl.ds(pl.multiple_of(i * RB, RB), RB)
        return pltpu.make_async_copy(xa_h.at[r, :], xa.at[r, :], sem_x.at[i])

    def wq_copy(n):
        c = pl.ds(n * D, D)
        return pltpu.make_async_copy(wqkv_h.at[:, c], wqkv.at[:, c], sem_w.at[n])

    w_copies = [
        pltpu.make_async_copy(bre_h, bcat.at[pl.ds(0, D), :], sem_w.at[3]),
        pltpu.make_async_copy(bim_h, bcat.at[pl.ds(D, D), :], sem_w.at[4]),
        pltpu.make_async_copy(xb_h, xb, sem_w.at[5]),
        pltpu.make_async_copy(cre_h, ccat.at[:, pl.ds(0, D)], sem_w.at[6]),
        pltpu.make_async_copy(cim_h, ccat.at[:, pl.ds(D, D)], sem_w.at[7]),
        pltpu.make_async_copy(wo_h, wo, sem_w.at[8]),
    ]
    x_copy(0).start()
    wq_copy(0).start()
    wq_copy(2).start()
    wq_copy(1).start()
    x_copy(1).start()

    zv[...] = jnp.zeros(zv.shape, I32)
    oT_prev[...] = jnp.zeros((128, NQ), BF16)
    kn_scr[...] = jnp.zeros(kn_scr.shape, F32)
    bad_scr[...] = jnp.zeros(bad_scr.shape, F32)
    sel[...] = jnp.where(lax.broadcasted_iota(I32, (128, HPG * 128), 0) // DH
                         == lax.broadcasted_iota(I32, (128, HPG * 128), 1) // 128, 1.0, 0.0).astype(BF16)
    u_scr[:, 0:8, :] = jnp.zeros((8, 8, 128), F32)
    h_scr[...] = jnp.zeros(h_scr.shape, F32)

    l_re = lre[...].astype(F32).reshape(1, D)
    l_im = lim[...].astype(F32).reshape(1, D)
    dt = jnp.exp(ldt[...].astype(F32).reshape(1, D)).astype(BF16).astype(F32)
    e_re = dt * l_re
    e_im = dt * l_im

    def apow(k):
        mag = jnp.exp(k * e_re)
        return mag * jnp.cos(k * e_im), mag * jnp.sin(k * e_im)

    a1r, a1i = apow(1.0)
    for n, k in enumerate((1.0, 2.0, 4.0, 8.0)):
        r, i = apow(k)
        coef[2 * n] = jnp.broadcast_to(r, (8, D))
        coef[2 * n + 1] = jnp.broadcast_to(i, (8, D))
    nr = a1r - 1.0
    den = l_re * l_re + l_im * l_im
    coef[8] = jnp.broadcast_to(2.0 * (nr * l_re + a1i * l_im) / den, (8, D))
    coef[9] = jnp.broadcast_to(2.0 * (a1i * l_re - nr * l_im) / den, (8, D))
    coef[10] = jnp.broadcast_to(dsk[...].astype(F32).reshape(1, D), (8, D))

    def proj_k(rows, xa_blk):
        kb = _nn(xa_blk, wqkv[:, D:2 * D])
        kbb = kb.astype(BF16)
        for g in range(NG):
            k_all[g, rows, :] = kbb[:, g * 128:(g + 1) * 128]
        k2 = jnp.max((kb * kb).reshape(RB // 8, 8, D), axis=0)
        for g in range(NG):
            kn_scr[g] = jnp.maximum(kn_scr[g], k2[:, g * 128:(g + 1) * 128])

    x_copy(0).wait()
    wq_copy(0).wait()
    q0 = (_nn(xa[0:RB, :], wqkv[:, 0:D]) * QSCALE).astype(BF16)
    wq_copy(2).wait()
    for i in range(2, NRB):
        x_copy(i).start()
    qT_all[0] = q0.T
    v0 = _nn(xa[0:RB, :], wqkv[:, 2 * D:3 * D]).astype(BF16)
    wq_copy(1).wait()
    for cp in w_copies:
        cp.start()
    vT_all[0] = v0.T
    proj_k(pl.ds(0, RB), xa[0:RB, :])

    def proj(i, carry):
        x_copy(i).wait()
        rows = pl.ds(pl.multiple_of(i * RB, RB), RB)
        xa_blk = xa[rows, :]
        qT_all[i] = (_nn(xa_blk, wqkv[:, 0:D]) * QSCALE).astype(BF16).T
        vT_all[i] = _nn(xa_blk, wqkv[:, 2 * D:3 * D]).astype(BF16).T
        proj_k(rows, xa_blk)
        return carry

    lax.fori_loop(1, NRB, proj, 0)

    for g in range(NG):
        k2 = jnp.broadcast_to(jnp.max(kn_scr[g], axis=0, keepdims=True) * (1.0 + 2.0 ** -6), (8, 128))
        ks = _nn(k2.astype(BF16), sel[...])
        for j in range(HPG):
            knb[HPG * g + j] = ks[:, j * 128:(j + 1) * 128]

    def load_group(g):
        kc[...] = k_all[g]
        gr = pl.ds(pl.multiple_of(g * 128, 128), 128)
        for b in range(NRB):
            vc[:, b * RB:(b + 1) * RB] = vT_all[b, gr, :]
        for n in range(NCK // 2):
            r0 = (2 * n + 1) * CK
            kf[n] = k_all[g, r0:r0 + 16, :].astype(F32)

    load_group(0)
    for cp in w_copies:
        cp.wait()

    def wmat(j):
        parts = []
        if j > 0:
            parts.append(jnp.zeros((DH * j, NQ), BF16))
        parts.append(wc[j * DH:(j + 1) * DH, :])
        if j < HPG - 1:
            parts.append(jnp.zeros((DH * (HPG - 1 - j), NQ), BF16))
        return jnp.concatenate(parts, axis=0)

    def y_copy(t):
        r = pl.ds(pl.multiple_of(t * SB, SB), SB)
        return pltpu.make_async_copy(y_stage.at[r, :], out.at[r, pl.ds(D, D)], sem_y.at[t])

    def a_copy(qb_):
        r = pl.ds(pl.multiple_of(qb_ * NQ, NQ), NQ)
        return pltpu.make_async_copy(a_stage.at[r, :], out.at[r, pl.ds(0, D)], sem_a.at[qb_])

    rowid = lax.broadcasted_iota(I32, (8, 128), 0)

    def ssm_scan(c):
        lanes = slice(c * 128, (c + 1) * 128)
        prev = {}

        def fir(ur, ui, halo):
            wr, wi = ur, ui
            for n, k in enumerate((1, 2, 4)):
                rr = pltpu.roll(wr, k, 0)
                ri = pltpu.roll(wi, k, 0)
                if halo:
                    sr, si = rr, ri
                else:
                    pr, pi = prev[n]
                    sr = jnp.where(rowid < k, pr, rr)
                    si = jnp.where(rowid < k, pi, ri)
                prev[n] = (rr, ri)
                if halo and n == 2:
                    break
                ar = coef[2 * n, :, lanes]
                ai = coef[2 * n + 1, :, lanes]
                wr, wi = wr + ar * sr - ai * si, wi + ar * si + ai * sr
            return wr, wi

        fir(u_scr[c, 0:8, :], u_scr[4 + c, 0:8, :], True)
        hr, hi = h_scr[c], h_scr[4 + c]
        outr, outi = [], []
        for tile in range(SB // 8):
            rows = slice(8 + tile * 8, 16 + tile * 8)
            wr, wi = fir(u_scr[c, rows, :], u_scr[4 + c, rows, :], False)
            ar = coef[6, :, lanes]
            ai = coef[7, :, lanes]
            hr, hi = wr + ar * hr - ai * hi, wi + ar * hi + ai * hr
            fr = coef[8, :, lanes]
            fi = coef[9, :, lanes]
            outr.append(fr * hr - fi * hi)
            outi.append(-(fr * hi + fi * hr))
        h_scr[c] = hr
        h_scr[4 + c] = hi
        u_scr[c, 0:8, :] = u_scr[c, SB:SB + 8, :]
        u_scr[4 + c, 0:8, :] = u_scr[4 + c, SB:SB + 8, :]
        return jnp.concatenate(outr, axis=0).astype(BF16), jnp.concatenate(outi, axis=0).astype(BF16)

    class VpuScores:
        def __init__(self, J):
            self.a, self.c, self.acc, self.d = J // NCK, J % NCK, None, 0

        def step(self, nd, gate):
            k16 = kf[self.c // 2] + jnp.concatenate([gate, gate], axis=0)
            for d in range(self.d, self.d + nd):
                col = DH * self.a + d
                kb = jnp.broadcast_to(k16[:, col:col + 1], (16, NQ))
                q8 = jnp.concatenate([jnp.broadcast_to(qf[ct, col:col + 1, :], (8, 128)) for ct in range(NT)], axis=1)
                tt = kb * jnp.concatenate([q8, q8], axis=0)
                self.acc = tt if self.acc is None else self.acc + tt
            self.d += nd

    def attn(t, carry):
        g = t // NQB
        qbi = t % NQB
        tp = jnp.maximum(t - 1, 0)

        @pl.when((qbi == 0) & (t > 0))
        def _():
            load_group(g)

        @pl.when(t == NB - 1)
        def _():
            rows = pl.ds((NQB - 2) * NQ, NQ)
            a_stage[rows, :] = a_stage[rows, :] + _tn(oT_prev[...], wo[(NG - 1) * 128:NG * 128, :])
            a_copy(NQB - 2).start()

        gr = pl.ds(pl.multiple_of(g * 128, 128), 128)
        wc[:, 0:RB] = qT_all[2 * qbi, gr, :]
        wc[:, RB:2 * RB] = qT_all[2 * qbi + 1, gr, :]
        for ct in range(NT):
            qf[ct] = wc[:, ct * 128:(ct + 1) * 128].astype(F32)

        srows = pl.ds(pl.multiple_of(t * SB, SB), SB)
        xb_blk = xb[srows, :]
        for c in range(4):
            bc = jnp.concatenate([bcat[c * 128:(c + 1) * 128, :], bcat[D + c * 128:D + (c + 1) * 128, :]], axis=0)
            uc = _nt(xb_blk, bc)
            u_scr[c, 8:8 + SB, :] = uc[:, 0:128]
            u_scr[4 + c, 8:8 + SB, :] = uc[:, 128:256]
        hs = [ssm_scan(c) for c in range(4)]

        zi = zv[...]

        def zgate(x):
            return lax.bitcast_convert_type(lax.bitcast_convert_type(x, I32) & zi, F32)

        def order(J):
            return [x for x in range(NKG - 1, -1, -1) if not (x == 0 and _on_vpu(J))]

        def dot_groups(J):
            a = J // NCK
            c = J % NCK
            stream = [(cc, x) for cc in range(NCK) for x in order(a * NCK + cc)]
            pos = [i for i in range(len(stream)) if i == 0 or stream[i - 1][0] != stream[i][0]]
            lo = 0 if c == 0 else pos[c] + SHIFT
            hi = len(stream) if c == NCK - 1 else pos[c + 1] + SHIFT
            return stream[lo:hi]

        def score_dot(J):
            lhs = jnp.concatenate([kc[c * CK + 16 * x:c * CK + 16 * (x + 1), :] for (c, x) in dot_groups(J)], axis=0)
            return _nn(lhs, wmat(J // NCK))

        def bound(j):
            q = jnp.concatenate([qf[ct, j * DH:(j + 1) * DH, :] for ct in range(NT)], axis=1)
            q2 = jnp.sum(q * q, axis=0, keepdims=True)
            kk = jnp.concatenate([knb[g * HPG + j][0:1]] * NT, axis=1)
            return jnp.broadcast_to(jnp.sqrt(q2 * kk), (8, NQ))

        def filler_ssm_out():
            hcat = jnp.concatenate([h[0] for h in hs] + [h[1] for h in hs], axis=1)
            y = _nt(hcat, ccat[...])
            skip = (xb_blk.astype(F32) * coef[10, 0:1, :]).astype(BF16).astype(F32)
            y_stage[srows, :] = y + skip

        def filler_attn_out():
            last = t == NB - 1
            p_rows = pl.ds(pl.multiple_of(jnp.where(last, NQB - 1, tp % NQB) * NQ, NQ), NQ)
            p_wo = wo[pl.ds(pl.multiple_of((tp // NQB) * 128, 128), 128), :]
            part = _tn(oT_prev[...], p_wo)
            a_stage[p_rows, :] = jnp.where(tp < NQB, 0.0, a_stage[p_rows, :]) + jnp.where(last, 0.0, part)

        st = {'bad': jnp.zeros((1, NQ), F32)}
        ps = {}
        units = {}

        def pv(J):
            a = J // NCK
            c = J % NCK
            pb = jnp.concatenate([ps.pop((c, x)) for x in range(NKG)], axis=0).astype(BF16)
            o = _nn(vc[a * DH:(a + 1) * DH, c * CK:(c + 1) * CK], pb)
            st[('o', a)] = o if c == 0 else st[('o', a)] + o
            if c == NCK - 1:
                lsum = jnp.sum(st.pop(('l', a)), axis=0, keepdims=True)
                oT_cur[a * DH:(a + 1) * DH, :] = (st.pop(('o', a)) / lsum).astype(BF16)
                st['bad'] = jnp.maximum(st['bad'], jnp.where(lsum >= L_SAFE, 0.0, 1.0))

        s_next = score_dot(0)
        for J in range(NJ):
            a = J // NCK
            c = J % NCK
            s = s_next
            if J + 1 < NJ:
                s_next = score_dot(J + 1)
            if c == NCK - 1:
                if J == NJ - 1:
                    filler_ssm_out()
                pv(J - 1)
            if J == NJ - 1:
                filler_attn_out()
            if c == BOUND_AT and a + 1 < HPG:
                m_next = bound(a + 1)
                m = m + jnp.concatenate([zgate(m_next[:, ct * 128:(ct + 1) * 128]) for ct in range(NT)], axis=1)
            if c == 0:
                m = bound(a) if a == 0 else m_next
                l = jnp.zeros((8, NQ), F32)
            for i, (cc, x) in enumerate(dot_groups(J)):
                sg = s[16 * i:16 * (i + 1)]
                p = jnp.exp2(sg.reshape(2, 8, NQ) - m[None])
                l = l + p[0] + p[1]
                ps[(cc, x)] = p.reshape(16, NQ)
                if i % 2 == 0:
                    gate = zgate(sg[0:8, 0:128])
                    for Ju in range(J + 1, min(J + VPU_SPAN, NJ - 1) + 1):
                        if _on_vpu(Ju):
                            if Ju not in units:
                                units[Ju] = VpuScores(Ju)
                            if units[Ju].d < DH:
                                units[Ju].step(min(VPU_DIMS, DH - units[Ju].d), gate)
                                break
            if _on_vpu(J):
                un = units.pop(J)
                if un.d < DH:
                    un.step(DH - un.d, gate)
                p = jnp.exp2(un.acc.reshape(2, 8, NQ) - m[None])
                l = l + p[0] + p[1]
                ps[(c, 0)] = p.reshape(16, NQ)
            st[('l', a)] = l
            if c != NCK - 2:
                pv(J)
        bad_scr[...] = jnp.maximum(bad_scr[...], st['bad'])
        oT_prev[...] = oT_cur[...]
        y_copy(t).start()

        @pl.when((t > (NG - 1) * NQB) & (t < NB - 1))
        def _():
            a_copy(tp % NQB).start()

        return carry

    lax.fori_loop(0, NB, attn, 0)

    wo_last = wo[(NG - 1) * 128:NG * 128, :]
    tail = []
    for n in range(4):
        r0 = (NQB - 1) * NQ + n * 128
        a_stage[r0:r0 + 128, :] = a_stage[r0:r0 + 128, :] + _tn(oT_prev[:, n * 128:(n + 1) * 128], wo_last)
        cp = pltpu.make_async_copy(a_stage.at[pl.ds(r0, 128), :], out.at[pl.ds(r0, 128), pl.ds(0, D)], sem_a.at[NQB - 1 + n])
        cp.start()
        tail.append(cp)

    for t in range(NB):
        y_copy(t).wait()
    for qb_ in range(NQB - 1):
        a_copy(qb_).wait()
    for cp in tail:
        cp.wait()

    @pl.when(jnp.max(bad_scr[...]) > 0.5)
    def _():
        headid = lax.broadcasted_iota(I32, (128, NQ), 0) // DH

        def fb_body(t, carry):
            g = t // NQB
            qbi = t % NQB
            gr = pl.ds(pl.multiple_of(g * 128, 128), 128)
            wc[:, 0:RB] = qT_all[2 * qbi, gr, :]
            wc[:, RB:2 * RB] = qT_all[2 * qbi + 1, gr, :]

            def fb_head(j, carry2):
                wj = jnp.where(headid == j, wc[...].astype(F32), 0.0).astype(BF16)

                def pass1(b, m):
                    rows = pl.ds(pl.multiple_of(b * RB, RB), RB)
                    s = _nn(k_all[g, rows, :], wj)
                    s_scr[rows, :] = s
                    return jnp.maximum(m, jnp.max(s, axis=0, keepdims=True))

                m = lax.fori_loop(0, NRB, pass1, jnp.full((1, NQ), -jnp.inf, F32))

                def pass2(b, lo):
                    rows = pl.ds(pl.multiple_of(b * RB, RB), RB)
                    p = jnp.exp2(s_scr[rows, :] - m)
                    hr = pl.ds(pl.multiple_of(g * 128 + j * DH, DH), DH)
                    return (lo[0] + jnp.sum(p, axis=0, keepdims=True),
                            lo[1] + _nn(vT_all[b, hr, :], p.astype(BF16)))

                l, o = lax.fori_loop(0, NRB, pass2, (jnp.zeros((1, NQ), F32), jnp.zeros((DH, NQ), F32)))
                oT_cur[pl.ds(pl.multiple_of(j * DH, DH), DH), :] = (o / l).astype(BF16)
                return carry2

            lax.fori_loop(0, HPG, fb_head, 0)
            rows = pl.ds(pl.multiple_of(qbi * NQ, NQ), NQ)
            part = _tn(oT_cur[...], wo[gr, :])
            a_stage[rows, :] = jnp.where(g == 0, 0.0, a_stage[rows, :]) + part
            return carry

        lax.fori_loop(0, NB, fb_body, 0)
        cps = [a_copy(qb_) for qb_ in range(NQB)]
        for cp in cps:
            cp.start()
        for cp in cps:
            cp.wait()


@jax.jit
def pallas_concat_heads__softmax_full_mha__ssm_conv_s5__prompt_kernel(
        A_x, A_wqkv, A_wo, B_x, B_Lambda_re, B_Lambda_im, B_B_re, B_B_im, B_C_re, B_C_im, B_log_dt, B_Dskip):
    xa = A_x.reshape(S, D)
    xb = B_x.reshape(S, D)
    vm = pl.BlockSpec(memory_space=pltpu.VMEM)
    hbm = pl.BlockSpec(memory_space=pl.ANY)
    out = pl.pallas_call(
        _kernel,
        out_shape=jax.ShapeDtypeStruct((S, 2 * D), F32),
        in_specs=[hbm, hbm, hbm, hbm, vm, vm, hbm, hbm, hbm, hbm, vm, vm],
        out_specs=hbm,
        scratch_shapes=[
            pltpu.VMEM((S, D), BF16),
            pltpu.VMEM((D, 3 * D), BF16),
            pltpu.VMEM((D, D), BF16),
            pltpu.VMEM((S, D), BF16),
            pltpu.VMEM((2 * D, D), BF16),
            pltpu.VMEM((D, 2 * D), BF16),
            pltpu.VMEM((11, 8, D), F32),
            pltpu.VMEM((NG, S, 128), BF16),
            pltpu.VMEM((NRB, D, RB), BF16),
            pltpu.VMEM((NRB, D, RB), BF16),
            pltpu.VMEM((128, NQ), BF16),
            pltpu.VMEM((128, NQ), BF16),
            pltpu.VMEM((S, 128), BF16),
            pltpu.VMEM((128, S), BF16),
            pltpu.VMEM((128, NQ), BF16),
            pltpu.VMEM((NCK // 2, 16, 128), F32),
            pltpu.VMEM((NT, 128, 128), F32),
            pltpu.VMEM((NG, 8, 128), F32),
            pltpu.VMEM((NG * HPG, 8, 128), F32),
            pltpu.VMEM((128, HPG * 128), BF16),
            pltpu.VMEM((1, NQ), F32),
            pltpu.VMEM((S, NQ), F32),
            pltpu.VMEM((8, 128), I32),
            pltpu.VMEM((8, SB + 8, 128), F32),
            pltpu.VMEM((8, 8, 128), F32),
            pltpu.VMEM((S, D), F32),
            pltpu.VMEM((S, D), F32),
            pltpu.SemaphoreType.DMA((9,)),
            pltpu.SemaphoreType.DMA((NRB,)),
            pltpu.SemaphoreType.DMA((NB,)),
            pltpu.SemaphoreType.DMA((NQB + 3,)),
        ],
        compiler_params=pltpu.CompilerParams(vmem_limit_bytes=100 * 2 ** 20),
        name="fused_mha_s5",
    )(xa, A_wqkv, A_wo, xb, B_Lambda_re, B_Lambda_im, B_B_re, B_B_im, B_C_re, B_C_im, B_log_dt, B_Dskip)
    return out.reshape(1, S, 2 * D)
```
